```python
import jax
import jax.numpy as jnp

def _softmax(x, axis=-1):
    return jax.nn.softmax(x, axis=axis)
def _gelu(x):
    return jax.nn.gelu(x, approximate=True)
def _silu(x):
    return jax.nn.silu(x)
def _sigmoid(x):
    return jax.nn.sigmoid(x)
def _layernorm(x, axis=-1, eps=1e-5):
    m = jnp.mean(x, axis=axis, keepdims=True)
    v = jnp.var(x, axis=axis, keepdims=True)
    return (x - m) / jnp.sqrt(v + eps)
def _scatter_add(tgt, idx, src, axis=0):
    return tgt.at[idx].add(src)
def _segment_sum(src, seg, n):
    return jax.ops.segment_sum(src, seg, n)
class _Rng:
    def __init__(self, key):
        self._k = key
    def _next(self):
        self._k, sub = jax.random.split(self._k)
        return sub
    def normal(self, shape):
        return jax.random.normal(self._next(), shape, dtype=jnp.bfloat16)
    def randint(self, lo, hi, shape):
        return jax.random.randint(self._next(), shape, lo, hi, dtype=jnp.int32)
    def uniform(self, shape, lo=0.0, hi=1.0):
        return jax.random.uniform(self._next(), shape, jnp.bfloat16, lo, hi)
    def permutation(self, n):
        return jax.random.permutation(self._next(), n)


kernel_name = 'gated_mix__compressed_kv_cla__gqa_block_cached__decode'

def setup_inputs():
    _rng = _Rng(jax.random.key(int.from_bytes(__import__("os").urandom(4), "little")))
    _w = (lambda a: (lambda t: t.astype(jnp.bfloat16) if jnp.issubdtype(t.dtype, jnp.floating) else t)(jnp.asarray(a)))
    def _A_setup():
        B, H, Sq, Sk, D, M = 1, 32, 1, 4096, 128, 640
        Dc = 4 * D
        return {
            "x": _w((lambda *s: _rng.normal(s) * 0.05)(B, Sq, M)),
            "c_kv": _w((lambda *s: _rng.normal(s) * 0.05)(B, Sk, Dc)),
            "w_q": _w((lambda *s: _rng.normal(s) * 0.05)(M, H, D) * (M ** -0.5)),
            "w_uk": _w((lambda *s: _rng.normal(s) * 0.05)(Dc, H, D) * (Dc ** -0.5)),
            "w_uv": _w((lambda *s: _rng.normal(s) * 0.05)(Dc, H, D) * (Dc ** -0.5)),
            "w_o": _w((lambda *s: _rng.normal(s) * 0.05)(H, D, M) * ((H * D) ** -0.5)),
        }
    _A_in = _A_setup()

    def _B_setup():
        B, Sq, D = 1, 1, 640
        Hq, Hkv, Sk, Dh = 32, 32, 4096, 128
        assert Hq % Hkv == 0, (Hq, Hkv)
        return {
            "x": _w((lambda *s: _rng.normal(s) * 0.05)(B, Sq, D)),
            "k_cache": _w((lambda *s: _rng.normal(s) * 0.05)(B, Hkv, Sk, Dh)),
            "v_cache": _w((lambda *s: _rng.normal(s) * 0.05)(B, Hkv, Sk, Dh)),
            "wq": _w((lambda *s: _rng.normal(s) * 0.05)(D, Hq * Dh) * (D ** -0.5)),
            "wo": _w((lambda *s: _rng.normal(s) * 0.05)(Hq * Dh, D) * ((Hq * Dh) ** -0.5)),
        }
    _B_in = _B_setup()

    return {
        "A_x": _A_in["x"],
        "A_c_kv": _A_in["c_kv"],
        "A_w_q": _A_in["w_q"],
        "A_w_uk": _A_in["w_uk"],
        "A_w_uv": _A_in["w_uv"],
        "A_w_o": _A_in["w_o"],
        "B_x": _B_in["x"],
        "B_k_cache": _B_in["k_cache"],
        "B_v_cache": _B_in["v_cache"],
        "B_wq": _B_in["wq"],
        "B_wo": _B_in["wo"],
        "gate_w": _w((lambda *s: _rng.normal(s) * 0.05)(640)),
    }

def reference(A_x, A_c_kv, A_w_q, A_w_uk, A_w_uv, A_w_o, B_x, B_k_cache, B_v_cache, B_wq, B_wo, gate_w):
    def _A_ref(x, c_kv, w_q, w_uk, w_uv, w_o):
        B, Sq, M = x.shape[0], x.shape[1], x.shape[2]
        Sk = c_kv.shape[1]
        H, D = w_q.shape[1], w_q.shape[2]
        q = jnp.einsum("bqm,mhd->bhqd", x, w_q)
        k = jnp.einsum("bkc,chd->bhkd", c_kv, w_uk)
        v = jnp.einsum("bkc,chd->bhkd", c_kv, w_uv)
        scores = jnp.einsum("bhqd,bhkd->bhqk", q, k) * (D ** -0.5)
        off = Sk - Sq
        qi = jnp.arange(Sq)[:, None]
        kj = jnp.arange(Sk)[None, :]
        cmask = kj <= (qi + off)
        scores = jnp.where(cmask[None, None], scores, -1e9)
        p = _softmax(scores, axis=-1)
        ctx = jnp.einsum("bhqk,bhkd->bhqd", p, v)
        return jnp.einsum("bhqd,hdm->bqm", ctx, w_o)

    def _B_ref(x, k_cache, v_cache, wq, wo):
        B, Sq, D = x.shape
        Hq, Dh = 32, 128
        Hkv = k_cache.shape[1]
        rep = Hq // Hkv
        q = (lambda x, *d: x.transpose(*d))((x @ wq).reshape(B, Sq, Hq, Dh), 0, 2, 1, 3)
        k = jnp.repeat(k_cache, rep, axis=1)
        v = jnp.repeat(v_cache, rep, axis=1)
        scores = jnp.einsum("bhqd,bhkd->bhqk", q, k) * (Dh ** -0.5)
        p = _softmax(scores, axis=-1)
        o = jnp.einsum("bhqk,bhkd->bhqd", p, v)
        return (lambda x, *d: x.transpose(*d))(o, 0, 2, 1, 3).reshape(B, Sq, Hq * Dh) @ wo

    x = A_x
    g = _sigmoid((x * gate_w).sum(-1, keepdims=True))
    a = _A_ref(x, A_c_kv, A_w_q, A_w_uk, A_w_uv, A_w_o)
    b = _B_ref(x, B_k_cache, B_v_cache, B_wq, B_wo)
    return g * a + (1 - g) * b
```

```python
import functools
import jax
import jax.numpy as jnp
from jax import lax
from jax.experimental import pallas as pl
from jax.experimental.pallas import tpu as pltpu

BF = jnp.bfloat16
F32 = jnp.float32
NT = (((1,), (1,)), ((), ()))
H = 32
SK = 4096
DEPTH = 3


def _unpack_pair(ref_u32, j, n):
    w = ref_u32[pl.ds(j, n, stride=16), :]
    lo = pltpu.bitcast(w << 16, F32).astype(BF)
    hi = pltpu.bitcast(w & jnp.uint32(0xFFFF0000), F32).astype(BF)
    return lo, hi


def kernel(x_hbm, gate_hbm, ckv_hbm, wq_hbm, wuk_hbm, wuv_hbm, wo_hbm, k_hbm, v_hbm, bwq_hbm, bwo_hbm,
           out_ref,
           x_v, gate_v, ckv_v, wq_v, wuk_v, wuv_v, wo_v, k_v, v_v, bwq_v, bwo_v,
           qa_s, qabs_s, s_s, p_s, ctxc_s, ctx_s, qb_s,
           sems, ksem, vsem):
    cp = lambda s, d, i: pltpu.make_async_copy(s, d, sems.at[i])
    c_x = cp(x_hbm, x_v, 0)
    c_g = cp(gate_hbm, gate_v, 1)
    c_wq = cp(wq_hbm, wq_v, 2)
    c_wuk = cp(wuk_hbm, wuk_v, 3)
    c_ckv = cp(ckv_hbm.at[0], ckv_v, 4)
    c_wuv = cp(wuv_hbm, wuv_v, 5)
    c_wo = cp(wo_hbm, wo_v, 6)
    c_bwq = cp(bwq_hbm, bwq_v, 7)
    c_bwo = cp(bwo_hbm, bwo_v, 8)
    kc = lambda h: pltpu.make_async_copy(k_hbm.at[0, h], k_v.at[h], ksem.at[h])
    vc = lambda h: pltpu.make_async_copy(v_hbm.at[0, h], v_v.at[h], vsem.at[h])

    c_x.start(); c_g.start(); c_wq.start(); c_wuk.start()
    c_x.wait(); c_g.wait()
    xf = x_v[0].astype(F32)
    x8 = jnp.broadcast_to(xf, (8, 640)).astype(BF)
    gf = gate_v[...].astype(F32).reshape(1, 640)
    prod = (xf * gf).astype(BF).astype(F32)
    gsum = jnp.sum(prod, axis=-1, keepdims=True)
    g = jax.nn.sigmoid(gsum)
    row8 = lax.broadcasted_iota(jnp.int32, (8, 128), 0)

    c_wq.wait(); c_ckv.start()
    wq_u = wq_v.bitcast(jnp.uint32)
    def a1(j, _):
        lo, hi = _unpack_pair(wq_u, j, 640)
        qa_s[2 * j] = jnp.dot(x8, lo, preferred_element_type=F32)
        qa_s[2 * j + 1] = jnp.dot(x8, hi, preferred_element_type=F32)
        return _
    for j in range(16): a1(j, 0)

    c_wuk.wait(); c_wuv.start()
    wuk_u = wuk_v.bitcast(jnp.uint32)
    qabs_s[...] = jnp.zeros(qabs_s.shape, F32)
    def a2(j, _):
        lo, hi = _unpack_pair(wuk_u, j, 512)
        h0 = 2 * j
        q0 = jnp.where(row8 == h0 % 8, qa_s[h0], 0.0).astype(BF)
        q1 = jnp.where(row8 == h0 % 8 + 1, qa_s[h0 + 1], 0.0).astype(BF)
        r = lax.dot_general(q0, lo, NT, preferred_element_type=F32) + \
            lax.dot_general(q1, hi, NT, preferred_element_type=F32)
        g_ = j // 4
        qabs_s[g_] = qabs_s[g_] + r
        return _
    for j in range(16): a2(j, 0)

    c_ckv.wait(); c_wo.start()
    qabs = qabs_s[...].reshape(32, 512).astype(BF)
    KC = 512
    def a3a(i, m):
        ck = ckv_v[pl.ds(pl.multiple_of(i * KC, KC), KC), :]
        s = lax.dot_general(qabs, ck, NT, preferred_element_type=F32) * (128 ** -0.5)
        s_s[:, pl.ds(pl.multiple_of(i * KC, KC), KC)] = s
        return jnp.maximum(m, jnp.max(s, axis=1, keepdims=True))
    m = lax.fori_loop(0, SK // KC, a3a, jnp.full((32, 1), -jnp.inf, F32))
    def a3b(i, carry):
        l, acc = carry
        sl = pl.ds(pl.multiple_of(i * KC, KC), KC)
        p = jnp.exp(s_s[:, sl] - m)
        l = l + jnp.sum(p, axis=1, keepdims=True)
        acc = acc + jnp.dot(p.astype(BF), ckv_v[sl, :], preferred_element_type=F32)
        return l, acc
    l, acc = lax.fori_loop(0, SK // KC, a3b, (jnp.zeros((32, 1), F32), jnp.zeros((32, 512), F32)))
    ctxc_s[...] = (acc / l).reshape(4, 8, 512)

    c_wuv.wait(); c_bwq.start()
    wuv_u = wuv_v.bitcast(jnp.uint32)
    row8b = lax.broadcasted_iota(jnp.int32, (8, 512), 0)
    def a4(j, _):
        lo, hi = _unpack_pair(wuv_u, j, 512)
        h0 = 2 * j
        cg = ctxc_s[j // 4]
        l0 = jnp.where(row8b == h0 % 8, cg, 0.0).astype(BF)
        l1 = jnp.where(row8b == h0 % 8 + 1, cg, 0.0).astype(BF)
        ctx_s[h0] = jnp.dot(l0, lo, preferred_element_type=F32)
        ctx_s[h0 + 1] = jnp.dot(l1, hi, preferred_element_type=F32)
        return _
    for j in range(16): a4(j, 0)

    c_wo.wait(); c_bwo.start()
    def a5(h, acc):
        return acc + jnp.dot(ctx_s[h].astype(BF), wo_v[h], preferred_element_type=F32)
    accA = lax.fori_loop(0, 32, a5, jnp.zeros((8, 640), F32))
    a_out = jnp.sum(accA, axis=0, keepdims=True)

    c_bwq.wait()
    for h in range(DEPTH):
        kc(h).start(); vc(h).start()
    qb = jnp.dot(x8, bwq_v[...], preferred_element_type=F32)
    for h in range(H):
        qb_s[h] = qb[:, h * 128:(h + 1) * 128]
    c_bwo.wait()

    def bh(h, acc):
        kc(h).wait()
        @pl.when(h + DEPTH < H)
        def _():
            kc(h + DEPTH).start(); vc(h + DEPTH).start()
        q = qb_s[h].astype(BF)
        s = lax.dot_general(q, k_v[h], NT, preferred_element_type=F32) * (128 ** -0.5)
        m = jnp.max(s, axis=1, keepdims=True)
        p = jnp.exp(s - m)
        l = jnp.sum(p, axis=1, keepdims=True)
        vc(h).wait()
        o = jnp.dot(p.astype(BF), v_v[h], preferred_element_type=F32) / l
        wo = bwo_v[pl.ds(pl.multiple_of(h * 128, 128), 128), :]
        return acc + jnp.dot(o.astype(BF), wo, preferred_element_type=F32)
    accB = lax.fori_loop(0, H, bh, jnp.zeros((8, 640), F32))
    b_out = accB[0:1, :]
    res = g * a_out + (1.0 - g) * b_out
    out_ref[0] = res.astype(out_ref.dtype)


@jax.jit
def pallas_gated_mix__compressed_kv_cla__gqa_block_cached__decode_kernel(A_x, A_c_kv, A_w_q, A_w_uk, A_w_uv, A_w_o, B_x, B_k_cache, B_v_cache, B_wq, B_wo, gate_w):
    any_spec = pl.BlockSpec(memory_space=pl.ANY)
    V = pltpu.VMEM
    return pl.pallas_call(
        kernel,
        in_specs=[any_spec] * 11,
        out_specs=pl.BlockSpec(memory_space=pltpu.VMEM),
        out_shape=jax.ShapeDtypeStruct((1, 1, 640), BF),
        scratch_shapes=[
            V((1, 1, 640), BF), V((640,), BF),
            V((4096, 512), BF), V((640 * 32, 128), BF), V((512 * 32, 128), BF), V((512 * 32, 128), BF),
            V((32, 128, 640), BF), V((32, 4096, 128), BF), V((32, 4096, 128), BF),
            V((640, 4096), BF), V((4096, 640), BF),
            V((32, 8, 128), F32), V((4, 8, 512), F32), V((32, 4096), F32), V((32, 4096), BF),
            V((4, 8, 512), F32), V((32, 8, 128), F32), V((32, 8, 128), F32),
            pltpu.SemaphoreType.DMA((9,)), pltpu.SemaphoreType.DMA((32,)), pltpu.SemaphoreType.DMA((32,)),
        ],
        compiler_params=pltpu.CompilerParams(vmem_limit_bytes=120 * 1024 * 1024),
    )(A_x, gate_w, A_c_kv, A_w_q.reshape(640 * 32, 128), A_w_uk.reshape(512 * 32, 128),
      A_w_uv.reshape(512 * 32, 128), A_w_o, B_k_cache, B_v_cache, B_wq, B_wo)
```

```python
import functools, contextlib
import jax
import jax.numpy as jnp
from jax import lax
from jax.experimental import pallas as pl
from jax.experimental.pallas import tpu as pltpu

BF = jnp.bfloat16
F32 = jnp.float32
I32 = jnp.int32
NT = (((1,), (1,)), ((), ()))
H = 32
SK = 4096
SCALE = 128 ** -0.5

S_X, S_G, S_WQ, S_BWQ, S_WUK, S_CKV, S_WUV, S_WO, S_BWO0 = range(9)

DEFAULT = dict(
    ns_p0=4, ns_p1=4, ns_p2=4, ns_bwo=4,
    t0=88,
    tgt=None,
    la1=96, la2=32, la_a=112,
    bwo_chunks=(2, 2, 2, 2),
    kvq=2, r_wo=32, r_bwo=32,
)

def rr_streams(n_streams, per_stream, mk):
  return [mk(s, k) for k in range(per_stream) for s in range(n_streams)]

def merge(a, b):
  out = []; ia = ib = 0
  while ia < len(a) or ib < len(b):
    if ib >= len(b) or (ia < len(a) and ia * len(b) <= ib * len(a)):
      out.append(a[ia]); ia += 1
    else:
      out.append(b[ib]); ib += 1
  return out


def make_kernel(compute=True, prof=False, cfg=None):
  cfg = dict(DEFAULT, **(cfg or {}))
  sc = (lambda n: jax.named_scope(n)) if prof else (lambda n: contextlib.nullcontext())
  NCH = len(cfg["bwo_chunks"])
  def kernel(x_hbm, gate_hbm, ckv_hbm, wq_hbm, wuk_hbm, wuv_hbm, wo_hbm, k_hbm, v_hbm, bwq_hbm, bwo_hbm,
             out_ref,
             x_v, gate_v, ckv_v, wq_v, wuk_v, wuv_v, wo_v, k_v, v_v, bwq_v, bwo_v,
             xe_s, s_s, ctx_s, qb_s, ob_s, qa_s, qabs4_s, m_s, ct4_s, a_s,
             sems, ksem, vsem):

    ndma = [0]
    def dma(src, dst, sem, prio=None):
      if prio is None:
        i = ndma[0]
        prio = (i + i // 2) % 2 if cfg.get("bal") else i % 2
      ndma[0] += 1
      pltpu.make_async_copy(src, dst, sem).start(priority=prio)

    def wait_all(buf, sem):
      pltpu.make_async_copy(buf, buf, sem).wait()

    def d_rows(hbm, vm, sem, nrows, ns):
      per = nrows // ns
      return rr_streams(ns, per // 128, lambda s, k: (lambda: dma(
          hbm.at[pl.ds(s * per + k * 128, 128)], vm.at[pl.ds(s * per + k * 128, 128)], sems.at[sem])))
    def d_bwq(ns):
      per = 640 // ns
      def mk(s, k):
        rr = pl.ds(s * per + (k // 2) * 8, 8); cc = pl.ds((k % 2) * 2048, 2048)
        return lambda: dma(bwq_hbm.at[rr, cc], bwq_v.at[rr, cc], sems.at[S_BWQ])
      return rr_streams(ns, (per // 8) * 2, mk)
    def d_ckv(ns):
      per = 4096 // ns
      return rr_streams(ns, per // 32, lambda s, k: (lambda: dma(
          ckv_hbm.at[0, pl.ds(s * per + k * 32, 32)], ckv_v.at[pl.ds(s * per + k * 32, 32)], sems.at[S_CKV])))
    def flat_plan(ns, R):
      per = 4096 // ns
      steps = []
      r0 = 0
      while r0 < per:
        n = min(R, per - r0); steps.append((r0, n)); r0 += n
      return per, steps
    def d_wo(ns, R):
      per, steps = flat_plan(ns, R)
      return rr_streams(ns, len(steps), lambda s, k: (lambda: dma(
          wo_hbm.at[pl.ds(s * per + steps[k][0], steps[k][1])],
          wo_v.at[pl.ds(s * per + steps[k][0], steps[k][1])], sems.at[S_WO])))
    def bwo_bounds(ns):
      hp = 32 // ns
      bounds = []; acc = 0
      for c in cfg["bwo_chunks"]:
        acc += c; bounds.append(acc)
      assert acc == hp
      return bounds
    def d_bwo(ns, R):
      per, steps = flat_plan(ns, R)
      bounds = bwo_bounds(ns)
      def chunk_of(k):
        last = steps[k][0] + steps[k][1] - 1
        return next(i for i, b in enumerate(bounds) if last // 128 < b)
      lst = rr_streams(ns, len(steps), lambda s, k: (lambda: dma(
          bwo_hbm.at[pl.ds(s * per + steps[k][0], steps[k][1])],
          bwo_v.at[pl.ds(s * per + steps[k][0], steps[k][1])], sems.at[S_BWO0 + chunk_of(k)])))
      rows_per_chunk = [0] * len(bounds)
      for k in range(len(steps)):
        rows_per_chunk[chunk_of(k)] += steps[k][1] * ns
      return lst, rows_per_chunk
    def d_kv(g):
      out = []
      Q = cfg["kvq"]; part = 4096 // Q
      for r in range(part // 128):
        for q in range(Q):
          rows = pl.ds(q * part + r * 128, 128)
          for hh in range(2):
            h = 2 * g + hh
            out.append(lambda rows=rows, h=h: dma(k_hbm.at[0, h, rows], k_v.at[h, rows], ksem.at[g], 0))
            out.append(lambda rows=rows, h=h: dma(v_hbm.at[0, h, rows], v_v.at[h, rows], vsem.at[g], 1))
      return out

    p0 = merge(d_rows(wq_hbm, wq_v, S_WQ, 20480, cfg["ns_p0"]), d_bwq(cfg["ns_p0"]))
    p1 = merge(d_rows(wuk_hbm, wuk_v, S_WUK, 16384, cfg["ns_p1"]), d_ckv(cfg["ns_p1"]))
    p2 = merge(d_rows(wuv_hbm, wuv_v, S_WUV, 16384, cfg["ns_p2"]), d_wo(cfg["ns_p2"], cfg["r_wo"]))
    def swap_pairs(lst, period):
      out = list(lst)
      for i in range(0, len(lst) - 1, 2):
        if (i // 2 // period) % 2 == 1:
          out[i], out[i + 1] = lst[i + 1], lst[i]
      return out
    if cfg.get("p2swap"):
      p2 = swap_pairs(p2, cfg["p2swap"])
    LA1, LA2 = cfg["la1"], cfg["la2"]
    g0 = d_kv(0)
    g1 = d_kv(1)
    E0 = len(p0); E1 = E0 + len(p1); E2 = E1 + len(p2); EG0 = E2 + 128
    static_list = p0 + p1 + p2 + g0 + g1[:LA1 + LA2]
    bwo_list, bwo_rows = d_bwo(cfg["ns_bwo"], cfg["r_bwo"])
    pos = [0]

    def issue_to(n):
      while pos[0] < min(n, len(static_list)):
        static_list[pos[0]]()
        pos[0] += 1

    c_x = pltpu.make_async_copy(x_hbm, x_v, sems.at[S_X])
    c_g = pltpu.make_async_copy(gate_hbm, gate_v, sems.at[S_G])
    c_x.start(); c_g.start()
    issue_to(cfg["t0"])
    c_x.wait(); c_g.wait()
    xf = x_v[0].astype(F32)
    x8 = jnp.broadcast_to(xf, (8, 640)).astype(BF)
    gf = gate_v[...].astype(F32).reshape(1, 640)
    prod = (xf * gf).astype(BF).astype(F32)
    g = jax.nn.sigmoid(jnp.sum(prod, axis=-1, keepdims=True))

    def iota(shape, d):
      return lax.broadcasted_iota(I32, shape, d)

    a_sel = jnp.where(iota((160, 640), 1) // 4 == iota((160, 640), 0),
                      jnp.broadcast_to(xf, (160, 640)), 0.0).astype(BF)
    b_sel = (iota((640, 128), 0) % 4 == iota((640, 128), 1) // 32).astype(F32).astype(BF)
    xe_s[...] = jnp.dot(a_sel, b_sel, preferred_element_type=F32)
    qa_s[...] = jnp.zeros(qa_s.shape, F32)
    qabs4_s[...] = jnp.zeros(qabs4_s.shape, F32)

    def mdiag():
      return iota((32, 128), 0) == iota((32, 128), 1) % 32

    def qa_part(i0, i1):
      md = mdiag()
      acc = qa_s[...]
      for it in range(i0, i1):
        T = wq_v[it * 1024:(it + 1) * 1024, :]
        xe8 = xe_s[it * 8:(it + 1) * 8, :]
        L = jnp.concatenate(
            [jnp.where(md, jnp.broadcast_to(xe8[tt:tt + 1, :], (32, 128)), 0.0).astype(BF) for tt in range(8)],
            axis=1)
        acc = acc + jnp.dot(L, T, preferred_element_type=F32)
      qa_s[...] = acc

    def qb_part():
      for c in range(4):
        qb = jnp.dot(x8, bwq_v[:, c * 1024:(c + 1) * 1024], preferred_element_type=F32)
        for hh in range(8):
          qb_s[c * 8 + hh] = qb[:, hh * 128:(hh + 1) * 128]

    def qabs_part(t0, t1):
      md = mdiag()
      dcol = iota((128, 128), 1) - iota((128, 128), 0) // 32
      q32 = qa_s[...].astype(BF)
      acc4 = qabs4_s[...]
      for tt in range(t0, t1):
        Rs = []
        for ch in range(4):
          T = wuk_v[ch * 4096 + tt * 128:ch * 4096 + (tt + 1) * 128, :]
          R = lax.dot_general(q32, T, NT, preferred_element_type=F32)
          Rs.append(jnp.where(md, R, 0.0).astype(BF))
        L4 = jnp.concatenate(Rs, axis=0)
        C = (dcol == 4 * tt).astype(F32).astype(BF)
        acc4 = acc4 + jnp.dot(L4, C, preferred_element_type=F32)
      qabs4_s[...] = acc4

    KC = 512
    def scores_part():
      acc4 = qabs4_s[...]
      qabs = jnp.concatenate([acc4[ch * 32:(ch + 1) * 32, :] for ch in range(4)], axis=1).astype(BF)
      m = jnp.full((32, 1), -jnp.inf, F32)
      for i in range(SK // KC):
        s = lax.dot_general(qabs, ckv_v[i * KC:(i + 1) * KC, :], NT, preferred_element_type=F32) * SCALE
        s_s[:, i * KC:(i + 1) * KC] = s
        m = jnp.maximum(m, jnp.max(s, axis=1, keepdims=True))
      m_s[...] = jnp.broadcast_to(m, (32, 128))

    def ctxc_part():
      m = m_s[:, 0:1]
      l = jnp.zeros((32, 1), F32)
      acc = jnp.zeros((32, 512), F32)
      for i in range(SK // KC):
        p = jnp.exp(s_s[:, i * KC:(i + 1) * KC] - m)
        l = l + jnp.sum(p, axis=1, keepdims=True)
        acc = acc + jnp.dot(p.astype(BF), ckv_v[i * KC:(i + 1) * KC, :], preferred_element_type=F32)
      ctxc = (acc / l).astype(BF)
      ct4_s[...] = jnp.concatenate([ctxc[:, ch * 128:(ch + 1) * 128] for ch in range(4)], axis=0)

    def ctx_part(t0, t1):
      md = mdiag()
      drow = iota((128, 128), 0) - iota((128, 128), 1) // 32
      CT4 = ct4_s[...]
      acc = jnp.zeros((32, 128), F32)
      for tt in range(t0, t1):
        E = (drow == 4 * tt).astype(F32).astype(BF)
        Z4 = jnp.dot(CT4, E, preferred_element_type=F32)
        for ch in range(4):
          L = jnp.where(md, Z4[ch * 32:(ch + 1) * 32, :], 0.0).astype(BF)
          T = wuv_v[ch * 4096 + tt * 128:ch * 4096 + (tt + 1) * 128, :]
          acc = acc + jnp.dot(L, T, preferred_element_type=F32)
      if t0 == 0:
        ctx_s[...] = acc.reshape(4, 8, 128)
      else:
        ctx_s[...] = ctx_s[...] + acc.reshape(4, 8, 128)

    def outa_part():
      row8 = iota((8, 128), 0)
      acc = jnp.zeros((8, 640), F32)
      for gi in range(4):
        cg = ctx_s[gi]
        L = jnp.concatenate([jnp.where(row8 == hh, cg, 0.0).astype(BF) for hh in range(8)], axis=1)
        W = wo_v[gi * 1024:(gi + 1) * 1024, :]
        acc = acc + jnp.dot(L, W, preferred_element_type=F32)
      a_s[...] = acc

    def head(h):
      if cfg.get("head_mode") == "dummy":
        x0 = ob_s[h]
        def bd(i, x):
          return jnp.exp(x * 0.001) * 0.5
        ob_s[h] = lax.fori_loop(0, cfg.get("dummy_n", 60), bd, x0)
        return
      q = qb_s[h].astype(BF)
      s = lax.dot_general(q, k_v[h], NT, preferred_element_type=F32) * SCALE
      m = jnp.max(s, axis=1, keepdims=True)
      p = jnp.exp(s - m)
      l = jnp.sum(p, axis=1, keepdims=True)
      ob_s[h] = jnp.dot(p.astype(BF), v_v[h], preferred_element_type=F32) / l

    def wait_p0():
      wait_all(wq_v, sems.at[S_WQ]); wait_all(bwq_v, sems.at[S_BWQ])
    def wait_p1():
      wait_all(wuk_v, sems.at[S_WUK]); wait_all(ckv_v, sems.at[S_CKV])
    def wait_p2():
      with sc('w_uv'):
        wait_all(wuv_v, sems.at[S_WUV])
      with sc('w_wo'):
        wait_all(wo_v, sems.at[S_WO])
    def wait_g0():
      with sc('w_k0'):
        wait_all(k_v.at[pl.ds(0, 2)], ksem.at[0])
      with sc('w_v0'):
        wait_all(v_v.at[pl.ds(0, 2)], vsem.at[0])

    def dummy_delay(n):
      def f():
        x0 = ob_s[0]
        ob_s[0] = lax.fori_loop(0, n, lambda i, x: jnp.exp(x * 0.001) * 0.5, x0)
      return f
    pieces = [
        (wait_p0, lambda: qa_part(0, 10)),
        (None, lambda: qa_part(10, 20)),
        (None, qb_part),
        (wait_p1, lambda: qabs_part(0, 16)),
        (None, lambda: qabs_part(16, 32)),
        (None, scores_part),
        (None, ctxc_part),
        (wait_p2, lambda: ctx_part(0, 16)),
        (None, lambda: ctx_part(16, 32)),
        (None, outa_part),
        (wait_g0, lambda: head(0)),
        (None, lambda: head(1)),
    ]
    LA = cfg.get("la_a", 80); S1 = cfg.get("step_a", 40); S2 = cfg.get("step_a2", 32)
    tgt = cfg["tgt"] or [E0 + LA, E0 + LA + S1, E0 + LA + 2 * S1, E1 + LA, E1 + LA + S1, E1 + LA + 2 * S1,
                         E1 + LA + 3 * S1, E2 + LA, E2 + LA + S2, E2 + LA + 2 * S2, EG0 + LA1, EG0 + LA1 + LA2]

    slots = []
    prev = cfg["t0"]
    for j, (w, piece) in enumerate(pieces):
      if cfg.get("split", True):
        for E in (E0, E1, E2, EG0):
          if prev < E < tgt[j]:
            slots.append((E, None, None, j))
      slots.append((tgt[j], w, piece, j))
      prev = max(prev, tgt[j])

    def stage(k, c):
      for n, (target, w, piece, j) in enumerate(slots):
        @pl.when(k == n)
        def _(n=n, target=target, w=w, piece=piece, j=j):
          with sc('p%02d_issue%s' % (j, '' if piece is not None else 'X')):
            issue_to(target)
          if w is not None:
            with sc('p%02d_wait' % j):
              w()
          if piece is not None and compute and (cfg.get('a_compute', True) or j >= 10) and (j in cfg.get('pieces', range(12))):
            with sc('p%02d_comp' % j):
              (dummy_delay(cfg['dummy'][j]) if j in cfg.get('dummy', {}) else pieces[cfg.get('remap', {}).get(j, j)][1])()
      return c
    lax.fori_loop(0, len(slots), stage, 0)
    assert pos[0] == len(static_list)

    nb = len(bwo_list)
    def bg(g, c):
      with sc('b_issue1'):
        cur = d_kv(g)
        for t in cur[LA1 + LA2:]:
          t()
        @pl.when(g + 1 < 16)
        def _():
          for t in d_kv(g + 1)[:LA1]:
            t()
        @pl.when(g == 15)
        def _():
          for t in bwo_list[:LA1]:
            t()
      with sc('b_wait'):
        wait_all(k_v.at[pl.ds(2 * g, 2)], ksem.at[g])
        wait_all(v_v.at[pl.ds(2 * g, 2)], vsem.at[g])
      with sc('b_head0'):
        if compute:
          head(2 * g)
      with sc('b_issue2'):
        @pl.when(g + 1 < 16)
        def _():
          for t in d_kv(g + 1)[LA1:LA1 + LA2]:
            t()
        @pl.when(g == 15)
        def _():
          for t in bwo_list[LA1:LA1 + LA2]:
            t()
      with sc('b_head1'):
        if compute:
          head(2 * g + 1)
      return c
    with sc('s10_Bloop'):
      lax.fori_loop(1, 16, bg, 0)

    with sc('s11_bwo'):
      for t in bwo_list[LA1 + LA2:]:
        t()
      accB = jnp.zeros((8, 640), F32)
      ns = cfg["ns_bwo"]; hp = 32 // ns
      h0 = 0
      for c, nh in enumerate(cfg["bwo_chunks"]):
        wait_all(bwo_v.at[pl.ds(0, bwo_rows[c])], sems.at[S_BWO0 + c])
        if compute:
          for s in range(ns):
            for hl in range(h0, h0 + nh):
              h = s * hp + hl
              accB = accB + jnp.dot(ob_s[h].astype(BF), bwo_v[h * 128:(h + 1) * 128, :], preferred_element_type=F32)
        h0 += nh
    b_out = accB[0:1, :]
    a_out = jnp.sum(a_s[...], axis=0, keepdims=True)
    res = g * a_out + (1.0 - g) * b_out
    out_ref[0] = res.astype(out_ref.dtype)
  kernel.nsem = S_BWO0 + NCH
  return kernel


def build(compute=True, prof=False, cfg=None):
  kern = make_kernel(compute, prof, cfg)
  @jax.jit
  def fn(A_x, A_c_kv, A_w_q, A_w_uk, A_w_uv, A_w_o, B_x, B_k_cache, B_v_cache, B_wq, B_wo, gate_w):
    any_spec = pl.BlockSpec(memory_space=pl.ANY)
    V = pltpu.VMEM
    return pl.pallas_call(
        kern,
        in_specs=[any_spec] * 11,
        out_specs=pl.BlockSpec(memory_space=pltpu.VMEM),
        out_shape=jax.ShapeDtypeStruct((1, 1, 640), BF),
        scratch_shapes=[
            V((1, 1, 640), BF), V((640,), BF),
            V((4096, 512), BF), V((640 * 32, 128), BF), V((512 * 32, 128), BF), V((512 * 32, 128), BF),
            V((4096, 640), BF), V((32, 4096, 128), BF), V((32, 4096, 128), BF),
            V((640, 4096), BF), V((4096, 640), BF),
            V((160, 128), F32), V((32, 4096), F32),
            V((4, 8, 128), F32), V((32, 8, 128), F32), V((32, 8, 128), F32),
            V((32, 128), F32), V((128, 128), F32), V((32, 128), F32),
            V((128, 128), BF), V((8, 640), F32),
            pltpu.SemaphoreType.DMA((kern.nsem,)), pltpu.SemaphoreType.DMA((16,)), pltpu.SemaphoreType.DMA((16,)),
        ],
        compiler_params=pltpu.CompilerParams(vmem_limit_bytes=120 * 1024 * 1024),
    )(A_x, gate_w, A_c_kv, A_w_q.reshape(640 * 32, 128), A_w_uk.reshape(512 * 32, 128),
      A_w_uv.reshape(512 * 32, 128), A_w_o.reshape(4096, 640), B_k_cache, B_v_cache, B_wq, B_wo)
  return fn

pallas_gated_mix__compressed_kv_cla__gqa_block_cached__decode_kernel = build(True)
```

```python
import functools, contextlib
import jax
import jax.numpy as jnp
from jax import lax
from jax.experimental import pallas as pl
from jax.experimental.pallas import tpu as pltpu

BF = jnp.bfloat16
F32 = jnp.float32
I32 = jnp.int32
NT = (((1,), (1,)), ((), ()))
H = 32
SK = 4096
SCALE = 128 ** -0.5

S_X, S_G, S_WQ, S_BWQ, S_WUK, S_CKV, S_WUV, S_WO, S_BWO0 = range(9)

DEFAULT = dict(
    ns_p0=4, ns_p1=4, ns_p2=4, ns_bwo=4,
    t0=88,
    tgt=None,
    la1=96, la2=32, la_a=112,
    bwo_chunks=(1, 1, 1, 1), modes="cccsc", wo_tile=(16, 128),
    kvq=2, r_wo=32, r_bwo=32,
)

def rr_streams(n_streams, per_stream, mk):
  return [mk(s, k) for k in range(per_stream) for s in range(n_streams)]

def merge(a, b):
  out = []; ia = ib = 0
  while ia < len(a) or ib < len(b):
    if ib >= len(b) or (ia < len(a) and ia * len(b) <= ib * len(a)):
      out.append(a[ia]); ia += 1
    else:
      out.append(b[ib]); ib += 1
  return out


def make_kernel(compute=True, prof=False, cfg=None):
  cfg = dict(DEFAULT, **(cfg or {}))
  sc = (lambda n: jax.named_scope(n)) if prof else (lambda n: contextlib.nullcontext())
  NCH = len(cfg["bwo_chunks"])
  def kernel(x_hbm, gate_hbm, ckv_hbm, wq_hbm, wuk_hbm, wuv_hbm, wo_hbm, k_hbm, v_hbm, bwq_hbm, bwo_hbm,
             out_ref,
             x_v, gate_v, ckv_v, wq_v, wuk_v, wuv_v, wo_v, k_v, v_v, bwq_v, bwo_v,
             xe_s, s_s, ctx_s, qb_s, ob_s, qa_s, qabs4_s, m_s, ct4_s, a_s,
             sems, ksem, vsem):

    ndma = [0]
    def dma(src, dst, sem, prio=None):
      if prio is None:
        i = ndma[0]
        prio = (i + i // 2) % 2 if cfg.get("bal") else i % 2
      ndma[0] += 1
      pltpu.make_async_copy(src, dst, sem).start(priority=prio)

    def wait_all(buf, sem):
      pltpu.make_async_copy(buf, buf, sem).wait()

    def seg_rows(hbm, vm2d, sem, nseg, R):
      vm = vm2d.reshape(nseg, vm2d.shape[0] // nseg, 128)
      n = vm.shape[1] // R
      return [(lambda k=k: dma(hbm.at[:, pl.ds(k * R, R)], vm.at[:, pl.ds(k * R, R)], sems.at[sem])) for k in range(n)]
    def d_bwq():
      vm = bwq_v.reshape(8, 80, 4096)
      out = []
      for r in range(10):
        for c in range(16):
          rr = pl.ds(r * 8, 8); cc = pl.ds(c * 256, 256)
          out.append(lambda rr=rr, cc=cc: dma(bwq_hbm.at[:, rr, cc], vm.at[:, rr, cc], sems.at[S_BWQ]))
      return out
    def d_ckv():
      vm = ckv_v.reshape(8, 512, 512)
      out = []
      for r in range(64):
        for c in range(2):
          rr = pl.ds(r * 8, 8); cc = pl.ds(c * 256, 256)
          out.append(lambda rr=rr, cc=cc: dma(ckv_hbm.at[:, rr, cc], vm.at[:, rr, cc], sems.at[S_CKV]))
      return out
    def d_640(hbm, vm2d, sem_of):
      vm = vm2d.reshape(8, 512, 640)
      RW, CW = cfg["wo_tile"]
      out = []
      for r in range(512 // RW):
        for c in range(640 // CW):
          rr = pl.ds(r * RW, RW); cc = pl.ds(c * CW, CW)
          out.append(lambda rr=rr, cc=cc, r=r: dma(hbm.at[:, rr, cc], vm.at[:, rr, cc], sem_of(r * RW)))
      return out
    def bwo_bounds():
      bounds = []; acc = 0
      for c in cfg["bwo_chunks"]:
        acc += c; bounds.append(acc)
      assert acc == 4
      return bounds
    def d_bwo():
      bounds = bwo_bounds()
      chunk_of = lambda row: next(i for i, b in enumerate(bounds) if row // 128 < b)
      if cfg["modes"][4] == "s":
        lst = d_640(bwo_hbm, bwo_v, lambda row: sems.at[S_BWO0 + chunk_of(row)])
      else:
        vm = bwo_v.reshape(8, 512, 640)
        lst = rr_streams(8, 16, lambda s, k: (lambda: dma(bwo_hbm.at[s, pl.ds(k * 32, 32)], vm.at[s, pl.ds(k * 32, 32)],
                                                        sems.at[S_BWO0 + chunk_of(k * 32)])))
      rows_per_chunk = [8 * 128 * c for c in cfg["bwo_chunks"]]
      return lst, rows_per_chunk
    k3 = k_v.reshape(64, 2048, 128)
    v3 = v_v.reshape(64, 2048, 128)
    def d_kv(g):
      out = []
      sg = pl.ds(4 * g, 4)
      for r in range(64):
        rows = pl.ds(r * 32, 32)
        out.append(lambda rows=rows: dma(k_hbm.at[sg, rows], k3.at[sg, rows], ksem.at[g], 0))
        out.append(lambda rows=rows: dma(v_hbm.at[sg, rows], v3.at[sg, rows], vsem.at[g], 1))
      return out

    def c_rows(hbm, vm2d, sem, nseg, ns, R=128):
      vm = vm2d.reshape(nseg, vm2d.shape[0] // nseg, 128)
      rows = vm.shape[1]; sp = nseg // ns; per = sp * rows // R
      def mk(s, k):
        seg = s * sp + (k * R) // rows; r0 = (k * R) % rows
        return lambda: dma(hbm.at[seg, pl.ds(r0, R)], vm.at[seg, pl.ds(r0, R)], sems.at[sem])
      return rr_streams(ns, per, mk)
    def c_bwq(ns):
      vm = bwq_v.reshape(8, 80, 4096); sp = 8 // ns
      def mk(s, k):
        t = k // 2; seg = s * sp + (t * 8) // 80; r0 = (t * 8) % 80
        rr = pl.ds(r0, 8); cc = pl.ds((k % 2) * 2048, 2048)
        return lambda: dma(bwq_hbm.at[seg, rr, cc], vm.at[seg, rr, cc], sems.at[S_BWQ])
      return rr_streams(ns, sp * 10 * 2, mk)
    def c_wide(hbm, vm2d, width, sem_of, ns, R):
      vm = vm2d.reshape(8, 512, width); sp = 8 // ns
      def mk(s, k):
        seg = s * sp + (k * R) // 512; r0 = (k * R) % 512
        return lambda: dma(hbm.at[seg, pl.ds(r0, R)], vm.at[seg, pl.ds(r0, R)], sem_of(s, k * R))
      return rr_streams(ns, sp * 512 // R, mk)
    M = cfg["modes"]
    p0 = (merge(seg_rows(wq_hbm, wq_v, S_WQ, 8, 16), d_bwq()) if M[0] == "s" else
          merge(c_rows(wq_hbm, wq_v, S_WQ, 8, 4), c_bwq(4)))
    p1 = (merge(seg_rows(wuk_hbm, wuk_v, S_WUK, 8, 16), d_ckv()) if M[1] == "s" else
          merge(c_rows(wuk_hbm, wuk_v, S_WUK, 8, 4), c_wide(ckv_hbm, ckv_v, 512, lambda s, r: sems.at[S_CKV], 4, 32)))
    if M[2] == "s":
      p2 = merge(seg_rows(wuv_hbm, wuv_v, S_WUV, 8, 16), d_640(wo_hbm, wo_v, lambda row: sems.at[S_WO]))
    elif M[2] == "m":
      p2 = merge(seg_rows(wuv_hbm, wuv_v, S_WUV, 8, 16), c_wide(wo_hbm, wo_v, 640, lambda s, r: sems.at[S_WO], 4, 32))
    else:
      p2 = merge(c_rows(wuv_hbm, wuv_v, S_WUV, 8, 4), c_wide(wo_hbm, wo_v, 640, lambda s, r: sems.at[S_WO], 4, 32))
    if M[3] == "c":
      def d_kv(g):
        out = []
        for r in range(16):
          for q in range(2):
            rows = pl.ds(r * 128, 128)
            for hh in range(2):
              sg = 4 * g + 2 * hh + q
              out.append(lambda rows=rows, sg=sg: dma(k_hbm.at[sg, rows], k3.at[sg, rows], ksem.at[g], 0))
              out.append(lambda rows=rows, sg=sg: dma(v_hbm.at[sg, rows], v3.at[sg, rows], vsem.at[g], 1))
        return out
    def swap_pairs(lst, period):
      out = list(lst)
      for i in range(0, len(lst) - 1, 2):
        if (i // 2 // period) % 2 == 1:
          out[i], out[i + 1] = lst[i + 1], lst[i]
      return out
    if cfg.get("p2swap"):
      p2 = swap_pairs(p2, cfg["p2swap"])
    LA1, LA2 = cfg["la1"], cfg["la2"]
    g0 = d_kv(0)
    g1 = d_kv(1)
    E0 = len(p0); E1 = E0 + len(p1); E2 = E1 + len(p2); EG0 = E2 + 128
    static_list = p0 + p1 + p2 + g0 + g1[:LA1 + LA2]
    bwo_list, bwo_rows = d_bwo()
    pos = [0]

    def issue_to(n):
      while pos[0] < min(n, len(static_list)):
        static_list[pos[0]]()
        pos[0] += 1

    c_x = pltpu.make_async_copy(x_hbm, x_v, sems.at[S_X])
    c_g = pltpu.make_async_copy(gate_hbm, gate_v, sems.at[S_G])
    c_x.start(); c_g.start()
    issue_to(cfg["t0"])
    c_x.wait(); c_g.wait()
    xf = x_v[0].astype(F32)
    x8 = jnp.broadcast_to(xf, (8, 640)).astype(BF)
    gf = gate_v[...].astype(F32).reshape(1, 640)
    prod = (xf * gf).astype(BF).astype(F32)
    g = jax.nn.sigmoid(jnp.sum(prod, axis=-1, keepdims=True))

    def iota(shape, d):
      return lax.broadcasted_iota(I32, shape, d)

    a_sel = jnp.where(iota((160, 640), 1) // 4 == iota((160, 640), 0),
                      jnp.broadcast_to(xf, (160, 640)), 0.0).astype(BF)
    b_sel = (iota((640, 128), 0) % 4 == iota((640, 128), 1) // 32).astype(F32).astype(BF)
    xe_s[...] = jnp.dot(a_sel, b_sel, preferred_element_type=F32)
    qa_s[...] = jnp.zeros(qa_s.shape, F32)
    qabs4_s[...] = jnp.zeros(qabs4_s.shape, F32)

    def mdiag():
      return iota((32, 128), 0) == iota((32, 128), 1) % 32

    def qa_part(i0, i1):
      md = mdiag()
      acc = qa_s[...]
      for it in range(i0, i1):
        T = wq_v[it * 1024:(it + 1) * 1024, :]
        xe8 = xe_s[it * 8:(it + 1) * 8, :]
        L = jnp.concatenate(
            [jnp.where(md, jnp.broadcast_to(xe8[tt:tt + 1, :], (32, 128)), 0.0).astype(BF) for tt in range(8)],
            axis=1)
        acc = acc + jnp.dot(L, T, preferred_element_type=F32)
      qa_s[...] = acc

    def qb_part():
      for c in range(4):
        qb = jnp.dot(x8, bwq_v[:, c * 1024:(c + 1) * 1024], preferred_element_type=F32)
        for hh in range(8):
          qb_s[c * 8 + hh] = qb[:, hh * 128:(hh + 1) * 128]

    def qabs_part(t0, t1):
      md = mdiag()
      dcol = iota((128, 128), 1) - iota((128, 128), 0) // 32
      q32 = qa_s[...].astype(BF)
      acc4 = qabs4_s[...]
      for tt in range(t0, t1):
        Rs = []
        for ch in range(4):
          T = wuk_v[ch * 4096 + tt * 128:ch * 4096 + (tt + 1) * 128, :]
          R = lax.dot_general(q32, T, NT, preferred_element_type=F32)
          Rs.append(jnp.where(md, R, 0.0).astype(BF))
        L4 = jnp.concatenate(Rs, axis=0)
        C = (dcol == 4 * tt).astype(F32).astype(BF)
        acc4 = acc4 + jnp.dot(L4, C, preferred_element_type=F32)
      qabs4_s[...] = acc4

    KC = 512
    def scores_part():
      acc4 = qabs4_s[...]
      qabs = jnp.concatenate([acc4[ch * 32:(ch + 1) * 32, :] for ch in range(4)], axis=1).astype(BF)
      m = jnp.full((32, 1), -jnp.inf, F32)
      for i in range(SK // KC):
        s = lax.dot_general(qabs, ckv_v[i * KC:(i + 1) * KC, :], NT, preferred_element_type=F32) * SCALE
        s_s[:, i * KC:(i + 1) * KC] = s
        m = jnp.maximum(m, jnp.max(s, axis=1, keepdims=True))
      m_s[...] = jnp.broadcast_to(m, (32, 128))

    def ctxc_part():
      m = m_s[:, 0:1]
      l = jnp.zeros((32, 1), F32)
      acc = jnp.zeros((32, 512), F32)
      for i in range(SK // KC):
        p = jnp.exp(s_s[:, i * KC:(i + 1) * KC] - m)
        l = l + jnp.sum(p, axis=1, keepdims=True)
        acc = acc + jnp.dot(p.astype(BF), ckv_v[i * KC:(i + 1) * KC, :], preferred_element_type=F32)
      ctxc = (acc / l).astype(BF)
      ct4_s[...] = jnp.concatenate([ctxc[:, ch * 128:(ch + 1) * 128] for ch in range(4)], axis=0)

    def ctx_part(t0, t1):
      md = mdiag()
      drow = iota((128, 128), 0) - iota((128, 128), 1) // 32
      CT4 = ct4_s[...]
      acc = jnp.zeros((32, 128), F32)
      for tt in range(t0, t1):
        E = (drow == 4 * tt).astype(F32).astype(BF)
        Z4 = jnp.dot(CT4, E, preferred_element_type=F32)
        for ch in range(4):
          L = jnp.where(md, Z4[ch * 32:(ch + 1) * 32, :], 0.0).astype(BF)
          T = wuv_v[ch * 4096 + tt * 128:ch * 4096 + (tt + 1) * 128, :]
          acc = acc + jnp.dot(L, T, preferred_element_type=F32)
      if t0 == 0:
        ctx_s[...] = acc.reshape(4, 8, 128)
      else:
        ctx_s[...] = ctx_s[...] + acc.reshape(4, 8, 128)

    def outa_part():
      row8 = iota((8, 128), 0)
      acc = jnp.zeros((8, 640), F32)
      for gi in range(4):
        cg = ctx_s[gi]
        L = jnp.concatenate([jnp.where(row8 == hh, cg, 0.0).astype(BF) for hh in range(8)], axis=1)
        W = wo_v[gi * 1024:(gi + 1) * 1024, :]
        acc = acc + jnp.dot(L, W, preferred_element_type=F32)
      a_s[...] = acc

    def head(h):
      if cfg.get("head_mode") == "dummy":
        x0 = ob_s[h]
        def bd(i, x):
          return jnp.exp(x * 0.001) * 0.5
        ob_s[h] = lax.fori_loop(0, cfg.get("dummy_n", 60), bd, x0)
        return
      q = qb_s[h].astype(BF)
      s = lax.dot_general(q, k_v[h], NT, preferred_element_type=F32) * SCALE
      m = jnp.max(s, axis=1, keepdims=True)
      p = jnp.exp(s - m)
      l = jnp.sum(p, axis=1, keepdims=True)
      ob_s[h] = jnp.dot(p.astype(BF), v_v[h], preferred_element_type=F32) / l

    def wait_p0():
      wait_all(wq_v, sems.at[S_WQ]); wait_all(bwq_v, sems.at[S_BWQ])
    def wait_p1():
      wait_all(wuk_v, sems.at[S_WUK]); wait_all(ckv_v, sems.at[S_CKV])
    def wait_p2():
      with sc('w_uv'):
        wait_all(wuv_v, sems.at[S_WUV])
      with sc('w_wo'):
        wait_all(wo_v, sems.at[S_WO])
    def wait_g0():
      with sc('w_k0'):
        wait_all(k_v.at[pl.ds(0, 2)], ksem.at[0])
      with sc('w_v0'):
        wait_all(v_v.at[pl.ds(0, 2)], vsem.at[0])

    def dummy_delay(n):
      def f():
        x0 = ob_s[0]
        ob_s[0] = lax.fori_loop(0, n, lambda i, x: jnp.exp(x * 0.001) * 0.5, x0)
      return f
    pieces = [
        (wait_p0, lambda: qa_part(0, 10)),
        (None, lambda: qa_part(10, 20)),
        (None, qb_part),
        (wait_p1, lambda: qabs_part(0, 16)),
        (None, lambda: qabs_part(16, 32)),
        (None, scores_part),
        (None, ctxc_part),
        (wait_p2, lambda: ctx_part(0, 16)),
        (None, lambda: ctx_part(16, 32)),
        (None, outa_part),
        (wait_g0, lambda: head(0)),
        (None, lambda: head(1)),
    ]
    LA = cfg.get("la_a", 80); S1 = cfg.get("step_a", 40); S2 = cfg.get("step_a2", 32)
    tgt = cfg["tgt"] or [E0 + LA, E0 + LA + S1, E0 + LA + 2 * S1, E1 + LA, E1 + LA + S1, E1 + LA + 2 * S1,
                         E1 + LA + 3 * S1, E2 + LA, E2 + LA + S2, E2 + LA + 2 * S2, EG0 + LA1, EG0 + LA1 + LA2]

    slots = []
    prev = cfg["t0"]
    for j, (w, piece) in enumerate(pieces):
      if cfg.get("split", True):
        for E in (E0, E1, E2, EG0):
          if prev < E < tgt[j]:
            slots.append((E, None, None, j))
      slots.append((tgt[j], w, piece, j))
      prev = max(prev, tgt[j])

    def stage(k, c):
      for n, (target, w, piece, j) in enumerate(slots):
        @pl.when(k == n)
        def _(n=n, target=target, w=w, piece=piece, j=j):
          with sc('p%02d_issue%s' % (j, '' if piece is not None else 'X')):
            issue_to(target)
          if w is not None:
            with sc('p%02d_wait' % j):
              w()
          if piece is not None and compute and (cfg.get('a_compute', True) or j >= 10) and (j in cfg.get('pieces', range(12))):
            with sc('p%02d_comp' % j):
              (dummy_delay(cfg['dummy'][j]) if j in cfg.get('dummy', {}) else pieces[cfg.get('remap', {}).get(j, j)][1])()
      return c
    lax.fori_loop(0, len(slots), stage, 0)
    assert pos[0] == len(static_list)

    nb = len(bwo_list)
    def bg(g, c):
      with sc('b_issue1'):
        cur = d_kv(g)
        for t in cur[LA1 + LA2:]:
          t()
        @pl.when(g + 1 < 16)
        def _():
          for t in d_kv(g + 1)[:LA1]:
            t()
        @pl.when(g == 15)
        def _():
          for t in bwo_list[:LA1]:
            t()
      with sc('b_wait'):
        wait_all(k_v.at[pl.ds(2 * g, 2)], ksem.at[g])
        wait_all(v_v.at[pl.ds(2 * g, 2)], vsem.at[g])
      with sc('b_head0'):
        if compute:
          head(2 * g)
      with sc('b_issue2'):
        @pl.when(g + 1 < 16)
        def _():
          for t in d_kv(g + 1)[LA1:LA1 + LA2]:
            t()
        @pl.when(g == 15)
        def _():
          for t in bwo_list[LA1:LA1 + LA2]:
            t()
      with sc('b_head1'):
        if compute:
          head(2 * g + 1)
      return c
    with sc('s10_Bloop'):
      lax.fori_loop(1, 16, bg, 0)

    with sc('s11_bwo'):
      for t in bwo_list[LA1 + LA2:]:
        t()
      accB = jnp.zeros((8, 640), F32)
      ns = 8; hp = 4
      h0 = 0
      for c, nh in enumerate(cfg["bwo_chunks"]):
        wait_all(bwo_v.at[pl.ds(0, bwo_rows[c])], sems.at[S_BWO0 + c])
        if compute:
          for s in range(ns):
            for hl in range(h0, h0 + nh):
              h = s * hp + hl
              accB = accB + jnp.dot(ob_s[h].astype(BF), bwo_v[h * 128:(h + 1) * 128, :], preferred_element_type=F32)
        h0 += nh
    b_out = accB[0:1, :]
    a_out = jnp.sum(a_s[...], axis=0, keepdims=True)
    res = g * a_out + (1.0 - g) * b_out
    out_ref[0] = res.astype(out_ref.dtype)
  kernel.nsem = S_BWO0 + NCH
  return kernel


def build(compute=True, prof=False, cfg=None):
  kern = make_kernel(compute, prof, cfg)
  @jax.jit
  def fn(A_x, A_c_kv, A_w_q, A_w_uk, A_w_uv, A_w_o, B_x, B_k_cache, B_v_cache, B_wq, B_wo, gate_w):
    any_spec = pl.BlockSpec(memory_space=pl.ANY)
    V = pltpu.VMEM
    return pl.pallas_call(
        kern,
        in_specs=[any_spec] * 11,
        out_specs=pl.BlockSpec(memory_space=pltpu.VMEM),
        out_shape=jax.ShapeDtypeStruct((1, 1, 640), BF),
        scratch_shapes=[
            V((1, 1, 640), BF), V((640,), BF),
            V((4096, 512), BF), V((640 * 32, 128), BF), V((512 * 32, 128), BF), V((512 * 32, 128), BF),
            V((4096, 640), BF), V((32, 4096, 128), BF), V((32, 4096, 128), BF),
            V((640, 4096), BF), V((4096, 640), BF),
            V((160, 128), F32), V((32, 4096), F32),
            V((4, 8, 128), F32), V((32, 8, 128), F32), V((32, 8, 128), F32),
            V((32, 128), F32), V((128, 128), F32), V((32, 128), F32),
            V((128, 128), BF), V((8, 640), F32),
            pltpu.SemaphoreType.DMA((kern.nsem,)), pltpu.SemaphoreType.DMA((16,)), pltpu.SemaphoreType.DMA((16,)),
        ],
        compiler_params=pltpu.CompilerParams(vmem_limit_bytes=120 * 1024 * 1024),
    )(A_x, gate_w, A_c_kv.reshape(8, 512, 512), A_w_q.reshape(8, 2560, 128), A_w_uk.reshape(8, 2048, 128),
      A_w_uv.reshape(8, 2048, 128), A_w_o.reshape(8, 512, 640), B_k_cache.reshape(64, 2048, 128),
      B_v_cache.reshape(64, 2048, 128), B_wq.reshape(8, 80, 4096), B_wo.reshape(8, 512, 640))
  return fn

pallas_gated_mix__compressed_kv_cla__gqa_block_cached__decode_kernel = build(True)
```

```python
import functools, contextlib
import jax
import jax.numpy as jnp
from jax import lax
from jax.experimental import pallas as pl
from jax.experimental.pallas import tpu as pltpu

BF = jnp.bfloat16
F32 = jnp.float32
I32 = jnp.int32
NT = (((1,), (1,)), ((), ()))
H = 32
SK = 4096
SCALE = 128 ** -0.5

S_X, S_G, S_WQ, S_BWQ, S_WUK, S_CKV, S_WUV, S_WO, S_BWO0 = range(9)

DEFAULT = dict(
    ns_p0=4, ns_p1=4, ns_p2=4, ns_bwo=4,
    t0=88,
    tgt=None,
    la1=96, la2=32, la_a=112,
    bwo_chunks=(1, 1, 1, 1), modes="cccsc", wo_tile=(16, 128),
    kvq=2, r_wo=32, r_bwo=32,
)

def rr_streams(n_streams, per_stream, mk):
  return [mk(s, k) for k in range(per_stream) for s in range(n_streams)]

def merge(a, b):
  out = []; ia = ib = 0
  while ia < len(a) or ib < len(b):
    if ib >= len(b) or (ia < len(a) and ia * len(b) <= ib * len(a)):
      out.append(a[ia]); ia += 1
    else:
      out.append(b[ib]); ib += 1
  return out


def make_kernel(compute=True, prof=False, cfg=None):
  cfg = dict(DEFAULT, **(cfg or {}))
  sc = (lambda n: jax.named_scope(n)) if prof else (lambda n: contextlib.nullcontext())
  NCH = len(cfg["bwo_chunks"])
  def kernel(x_hbm, gate_hbm, ckv_hbm, wq_hbm, wuk_hbm, wuv_hbm, wo_hbm, k_hbm, v_hbm, bwq_hbm, bwo_hbm,
             out_ref,
             x_v, gate_v, ckv_v, wq_v, wuk_v, wuv_v, wo_v, k_v, v_v, bwq_v, bwo_v,
             xe_s, s_s, ctx_s, qb_s, ob_s, qa_s, qabs4_s, m_s, ct4_s, a_s, accb_s,
             sems, ksem, vsem):

    ndma = [0]
    def dma(src, dst, sem, prio=None):
      if prio is None:
        i = ndma[0]
        prio = (i + i // 2) % 2 if cfg.get("bal") else i % 2
      ndma[0] += 1
      pltpu.make_async_copy(src, dst, sem).start(priority=prio)

    def wait_all(buf, sem):
      pltpu.make_async_copy(buf, buf, sem).wait()

    def seg_rows(hbm, vm2d, sem, nseg, R):
      vm = vm2d.reshape(nseg, vm2d.shape[0] // nseg, 128)
      n = vm.shape[1] // R
      return [(lambda k=k: dma(hbm.at[:, pl.ds(k * R, R)], vm.at[:, pl.ds(k * R, R)], sems.at[sem])) for k in range(n)]
    def d_bwq():
      vm = bwq_v.reshape(8, 80, 4096)
      out = []
      for r in range(10):
        for c in range(16):
          rr = pl.ds(r * 8, 8); cc = pl.ds(c * 256, 256)
          out.append(lambda rr=rr, cc=cc: dma(bwq_hbm.at[:, rr, cc], vm.at[:, rr, cc], sems.at[S_BWQ]))
      return out
    def d_ckv():
      vm = ckv_v.reshape(8, 512, 512)
      out = []
      for r in range(64):
        for c in range(2):
          rr = pl.ds(r * 8, 8); cc = pl.ds(c * 256, 256)
          out.append(lambda rr=rr, cc=cc: dma(ckv_hbm.at[:, rr, cc], vm.at[:, rr, cc], sems.at[S_CKV]))
      return out
    def d_640(hbm, vm2d, sem_of):
      vm = vm2d.reshape(8, 512, 640)
      RW, CW = cfg["wo_tile"]
      out = []
      for r in range(512 // RW):
        for c in range(640 // CW):
          rr = pl.ds(r * RW, RW); cc = pl.ds(c * CW, CW)
          out.append(lambda rr=rr, cc=cc, r=r: dma(hbm.at[:, rr, cc], vm.at[:, rr, cc], sem_of(r * RW)))
      return out
    def bwo_bounds():
      bounds = []; acc = 0
      for c in cfg["bwo_chunks"]:
        acc += c; bounds.append(acc)
      assert acc == 4
      return bounds
    def d_bwo():
      bounds = bwo_bounds()
      chunk_of = lambda row: next(i for i, b in enumerate(bounds) if row // 128 < b)
      if cfg["modes"][4] == "s":
        lst = d_640(bwo_hbm, bwo_v, lambda row: sems.at[S_BWO0 + chunk_of(row)])
      else:
        vm = bwo_v.reshape(8, 512, 640)
        lst = rr_streams(8, 16, lambda s, k: (lambda: dma(bwo_hbm.at[s, pl.ds(k * 32, 32)], vm.at[s, pl.ds(k * 32, 32)],
                                                        sems.at[S_BWO0 + chunk_of(k * 32)])))
      rows_per_chunk = [8 * 128 * c for c in cfg["bwo_chunks"]]
      return lst, rows_per_chunk
    def d_kv8(G, i0, n):
      out = []
      sg = pl.ds(8 * G, 8) if isinstance(G, int) else pl.ds(pl.multiple_of(8 * G, 8), 8)
      for i in range(n):
        r0 = (i0 + i) * 16
        rows = pl.ds(r0, 16) if isinstance(r0, int) else pl.ds(pl.multiple_of(r0, 16), 16)
        out.append(lambda rows=rows: dma(k_hbm.at[sg, rows], k_v.at[sg, rows], ksem.at[G], 0))
        out.append(lambda rows=rows: dma(v_hbm.at[sg, rows], v_v.at[sg, rows], vsem.at[G], 1))
      return out

    k64_hbm = k_hbm.reshape(64, 2048, 128); v64_hbm = v_hbm.reshape(64, 2048, 128)
    k64 = k_v.reshape(64, 2048, 128); v64 = v_v.reshape(64, 2048, 128)
    def d_kv2(g, i0, n, semi):
      out = []
      sg = pl.ds(pl.multiple_of(4 * g, 4), 4)
      for i in range(n):
        rows = pl.ds(pl.multiple_of((i0 + i) * 32, 32), 32)
        out.append(lambda rows=rows: dma(k64_hbm.at[sg, rows], k64.at[sg, rows], ksem.at[semi], 0))
        out.append(lambda rows=rows: dma(v64_hbm.at[sg, rows], v64.at[sg, rows], vsem.at[semi], 1))
      return out

    def c_rows(hbm, vm2d, sem, nseg, ns, R=128):
      vm = vm2d.reshape(nseg, vm2d.shape[0] // nseg, 128)
      rows = vm.shape[1]; sp = nseg // ns; per = sp * rows // R
      def mk(s, k):
        seg = s * sp + (k * R) // rows; r0 = (k * R) % rows
        return lambda: dma(hbm.at[seg, pl.ds(r0, R)], vm.at[seg, pl.ds(r0, R)], sems.at[sem])
      return rr_streams(ns, per, mk)
    def c_bwq(ns):
      vm = bwq_v.reshape(8, 80, 4096); sp = 8 // ns
      def mk(s, k):
        t = k // 2; seg = s * sp + (t * 8) // 80; r0 = (t * 8) % 80
        rr = pl.ds(r0, 8); cc = pl.ds((k % 2) * 2048, 2048)
        return lambda: dma(bwq_hbm.at[seg, rr, cc], vm.at[seg, rr, cc], sems.at[S_BWQ])
      return rr_streams(ns, sp * 10 * 2, mk)
    def c_wide(hbm, vm2d, width, sem_of, ns, R):
      vm = vm2d.reshape(8, 512, width); sp = 8 // ns
      def mk(s, k):
        seg = s * sp + (k * R) // 512; r0 = (k * R) % 512
        return lambda: dma(hbm.at[seg, pl.ds(r0, R)], vm.at[seg, pl.ds(r0, R)], sem_of(s, k * R))
      return rr_streams(ns, sp * 512 // R, mk)
    M = cfg["modes"]
    p0 = (merge(seg_rows(wq_hbm, wq_v, S_WQ, 8, 16), d_bwq()) if M[0] == "s" else
          merge(c_rows(wq_hbm, wq_v, S_WQ, 8, 4), c_bwq(4)))
    p1 = (merge(seg_rows(wuk_hbm, wuk_v, S_WUK, 8, 16), d_ckv()) if M[1] == "s" else
          merge(c_rows(wuk_hbm, wuk_v, S_WUK, 8, 4), c_wide(ckv_hbm, ckv_v, 512, lambda s, r: sems.at[S_CKV], 4, 32)))
    if M[2] == "s":
      p2 = merge(seg_rows(wuv_hbm, wuv_v, S_WUV, 8, 16), d_640(wo_hbm, wo_v, lambda row: sems.at[S_WO]))
    elif M[2] == "m":
      p2 = merge(seg_rows(wuv_hbm, wuv_v, S_WUV, 8, 16), c_wide(wo_hbm, wo_v, 640, lambda s, r: sems.at[S_WO], 4, 32))
    else:
      p2 = merge(c_rows(wuv_hbm, wuv_v, S_WUV, 8, 4), c_wide(wo_hbm, wo_v, 640, lambda s, r: sems.at[S_WO], 4, 32))
    def swap_pairs(lst, period):
      out = list(lst)
      for i in range(0, len(lst) - 1, 2):
        if (i // 2 // period) % 2 == 1:
          out[i], out[i + 1] = lst[i + 1], lst[i]
      return out
    if cfg.get("p2swap"):
      p2 = swap_pairs(p2, cfg["p2swap"])
    LA1, LA2 = cfg["la1"], cfg["la2"]
    g0 = d_kv8(0, 0, 256)
    E0 = len(p0); E1 = E0 + len(p1); E2 = E1 + len(p2); EG0 = E2 + 512
    static_list = p0 + p1 + p2 + g0
    pos = [0]

    def issue_to(n):
      while pos[0] < min(n, len(static_list)):
        static_list[pos[0]]()
        pos[0] += 1

    c_x = pltpu.make_async_copy(x_hbm, x_v, sems.at[S_X])
    c_g = pltpu.make_async_copy(gate_hbm, gate_v, sems.at[S_G])
    c_x.start(); c_g.start()
    issue_to(cfg["t0"])
    c_x.wait(); c_g.wait()
    xf = x_v[0].astype(F32)
    x8 = jnp.broadcast_to(xf, (8, 640)).astype(BF)
    gf = gate_v[...].astype(F32).reshape(1, 640)
    prod = (xf * gf).astype(BF).astype(F32)
    g = jax.nn.sigmoid(jnp.sum(prod, axis=-1, keepdims=True))

    def iota(shape, d):
      return lax.broadcasted_iota(I32, shape, d)

    a_sel = jnp.where(iota((160, 640), 1) // 4 == iota((160, 640), 0),
                      jnp.broadcast_to(xf, (160, 640)), 0.0).astype(BF)
    b_sel = (iota((640, 128), 0) % 4 == iota((640, 128), 1) // 32).astype(F32).astype(BF)
    xe_s[...] = jnp.dot(a_sel, b_sel, preferred_element_type=F32)
    qa_s[...] = jnp.zeros(qa_s.shape, F32)
    qabs4_s[...] = jnp.zeros(qabs4_s.shape, F32)

    def mdiag():
      return iota((32, 128), 0) == iota((32, 128), 1) % 32

    def qa_part(i0, i1):
      md = mdiag()
      acc = qa_s[...]
      for it in range(i0, i1):
        T = wq_v[it * 1024:(it + 1) * 1024, :]
        xe8 = xe_s[it * 8:(it + 1) * 8, :]
        L = jnp.concatenate(
            [jnp.where(md, jnp.broadcast_to(xe8[tt:tt + 1, :], (32, 128)), 0.0).astype(BF) for tt in range(8)],
            axis=1)
        acc = acc + jnp.dot(L, T, preferred_element_type=F32)
      qa_s[...] = acc

    def qb_part():
      for c in range(4):
        qb = jnp.dot(x8, bwq_v[:, c * 1024:(c + 1) * 1024], preferred_element_type=F32)
        for hh in range(8):
          qb_s[c * 8 + hh] = qb[:, hh * 128:(hh + 1) * 128]

    def qabs_part(t0, t1):
      md = mdiag()
      dcol = iota((128, 128), 1) - iota((128, 128), 0) // 32
      q32 = qa_s[...].astype(BF)
      acc4 = qabs4_s[...]
      for tt in range(t0, t1):
        Rs = []
        for ch in range(4):
          T = wuk_v[ch * 4096 + tt * 128:ch * 4096 + (tt + 1) * 128, :]
          R = lax.dot_general(q32, T, NT, preferred_element_type=F32)
          Rs.append(jnp.where(md, R, 0.0).astype(BF))
        L4 = jnp.concatenate(Rs, axis=0)
        C = (dcol == 4 * tt).astype(F32).astype(BF)
        acc4 = acc4 + jnp.dot(L4, C, preferred_element_type=F32)
      qabs4_s[...] = acc4

    KC = 512
    def scores_part():
      acc4 = qabs4_s[...]
      qabs = jnp.concatenate([acc4[ch * 32:(ch + 1) * 32, :] for ch in range(4)], axis=1).astype(BF)
      m = jnp.full((32, 1), -jnp.inf, F32)
      for i in range(SK // KC):
        s = lax.dot_general(qabs, ckv_v[i * KC:(i + 1) * KC, :], NT, preferred_element_type=F32) * SCALE
        s_s[:, i * KC:(i + 1) * KC] = s
        m = jnp.maximum(m, jnp.max(s, axis=1, keepdims=True))
      m_s[...] = jnp.broadcast_to(m, (32, 128))

    def ctxc_part():
      m = m_s[:, 0:1]
      l = jnp.zeros((32, 1), F32)
      acc = jnp.zeros((32, 512), F32)
      for i in range(SK // KC):
        p = jnp.exp(s_s[:, i * KC:(i + 1) * KC] - m)
        l = l + jnp.sum(p, axis=1, keepdims=True)
        acc = acc + jnp.dot(p.astype(BF), ckv_v[i * KC:(i + 1) * KC, :], preferred_element_type=F32)
      ctxc = (acc / l).astype(BF)
      ct4_s[...] = jnp.concatenate([ctxc[:, ch * 128:(ch + 1) * 128] for ch in range(4)], axis=0)

    def ctx_part(t0, t1):
      md = mdiag()
      drow = iota((128, 128), 0) - iota((128, 128), 1) // 32
      CT4 = ct4_s[...]
      acc = jnp.zeros((32, 128), F32)
      for tt in range(t0, t1):
        E = (drow == 4 * tt).astype(F32).astype(BF)
        Z4 = jnp.dot(CT4, E, preferred_element_type=F32)
        for ch in range(4):
          L = jnp.where(md, Z4[ch * 32:(ch + 1) * 32, :], 0.0).astype(BF)
          T = wuv_v[ch * 4096 + tt * 128:ch * 4096 + (tt + 1) * 128, :]
          acc = acc + jnp.dot(L, T, preferred_element_type=F32)
      if t0 == 0:
        ctx_s[...] = acc.reshape(4, 8, 128)
      else:
        ctx_s[...] = ctx_s[...] + acc.reshape(4, 8, 128)

    def outa_part():
      row8 = iota((8, 128), 0)
      acc = jnp.zeros((8, 640), F32)
      for gi in range(4):
        cg = ctx_s[gi]
        L = jnp.concatenate([jnp.where(row8 == hh, cg, 0.0).astype(BF) for hh in range(8)], axis=1)
        W = wo_v[gi * 1024:(gi + 1) * 1024, :]
        acc = acc + jnp.dot(L, W, preferred_element_type=F32)
      a_s[...] = acc

    def head(h):
      if cfg.get("head_mode") == "dummy":
        x0 = ob_s[h]
        def bd(i, x):
          return jnp.exp(x * 0.001) * 0.5
        ob_s[h] = lax.fori_loop(0, cfg.get("dummy_n", 60), bd, x0)
        return
      q = qb_s[h].astype(BF)
      s = lax.dot_general(q, k_v[h], NT, preferred_element_type=F32) * SCALE
      m = jnp.max(s, axis=1, keepdims=True)
      p = jnp.exp(s - m)
      l = jnp.sum(p, axis=1, keepdims=True)
      ob_s[h] = jnp.dot(p.astype(BF), v_v[h], preferred_element_type=F32) / l

    def wait_p0():
      wait_all(wq_v, sems.at[S_WQ]); wait_all(bwq_v, sems.at[S_BWQ])
    def wait_p1():
      wait_all(wuk_v, sems.at[S_WUK]); wait_all(ckv_v, sems.at[S_CKV])
    def wait_p2():
      with sc('w_uv'):
        wait_all(wuv_v, sems.at[S_WUV])
      with sc('w_wo'):
        wait_all(wo_v, sems.at[S_WO])
    def wait_g0():
      with sc('w_k0'):
        wait_all(k_v.at[pl.ds(0, 2)], ksem.at[0])
      with sc('w_v0'):
        wait_all(v_v.at[pl.ds(0, 2)], vsem.at[0])

    def dummy_delay(n):
      def f():
        x0 = ob_s[0]
        ob_s[0] = lax.fori_loop(0, n, lambda i, x: jnp.exp(x * 0.001) * 0.5, x0)
      return f
    pieces = [
        (wait_p0, lambda: qa_part(0, 10)),
        (None, lambda: qa_part(10, 20)),
        (None, qb_part),
        (wait_p1, lambda: qabs_part(0, 16)),
        (None, lambda: qabs_part(16, 32)),
        (None, scores_part),
        (None, ctxc_part),
        (wait_p2, lambda: ctx_part(0, 16)),
        (None, lambda: ctx_part(16, 32)),
        (None, outa_part),
        (None, lambda: None),
    ]
    LA = cfg.get("la_a", 80); S1 = cfg.get("step_a", 40); S2 = cfg.get("step_a2", 32)
    tgt = cfg["tgt"] or [E0 + LA, E0 + LA + S1, E0 + LA + 2 * S1, E1 + LA, E1 + LA + S1, E1 + LA + 2 * S1,
                         E1 + LA + 3 * S1, E2 + LA, E2 + LA + S2, E2 + LA + 2 * S2, EG0]

    slots = []
    prev = cfg["t0"]
    for j, (w, piece) in enumerate(pieces):
      if cfg.get("split", True):
        for E in (E0, E1, E2, EG0):
          if prev < E < tgt[j]:
            slots.append((E, None, None, j))
      slots.append((tgt[j], w, piece, j))
      prev = max(prev, tgt[j])

    def stage(k, c):
      for n, (target, w, piece, j) in enumerate(slots):
        @pl.when(k == n)
        def _(n=n, target=target, w=w, piece=piece, j=j):
          with sc('p%02d_issue%s' % (j, '' if piece is not None else 'X')):
            issue_to(target)
          if w is not None:
            with sc('p%02d_wait' % j):
              w()
          if piece is not None and compute and (cfg.get('a_compute', True) or j >= 10) and (j in cfg.get('pieces', range(12))):
            with sc('p%02d_comp' % j):
              (dummy_delay(cfg['dummy'][j]) if j in cfg.get('dummy', {}) else pieces[cfg.get('remap', {}).get(j, j)][1])()
      return c
    lax.fori_loop(0, len(slots), stage, 0)
    assert pos[0] == len(static_list)

    bwo3 = bwo_v.reshape(8, 512, 640)
    def bwo_steps(k0, k1):
      for k in range(k0, k1):
        for s in range(8):
          dma(bwo_hbm.at[s, pl.ds(k * 32, 32)], bwo3.at[s, pl.ds(k * 32, 32)], sems.at[S_BWO0 + k // 4], s % 2)

    a_s2 = accb_s
    a_s2[...] = jnp.zeros(a_s2.shape, F32)
    BW0 = cfg.get("bw_sched", (8, 4, 4))

    BW0 = cfg.get("bw_sched", (8, 8))
    NST = 24 + len(BW0)

    def bh(h, c):
      G = h // 8
      hh = h % 8
      with sc('b_issue1'):
        @pl.when(h < 16)
        def _():
          for t in d_kv8(G + 1, hh * 32, 32):
            t()
        @pl.when((h >= 16) & (h < 24))
        def _():
          j = h - 16
          for t in d_kv2(12 + j // 2, (j % 2) * 32, 32, 3 + j // 2):
            t()
        k0 = 0
        for n_, nk in enumerate(BW0):
          @pl.when(h == 24 + n_)
          def _(k0=k0, nk=nk):
            bwo_steps(k0, k0 + nk)
          k0 += nk
      with sc('b_wait'):
        @pl.when((hh == 0) & (h < 24))
        def _():
          wait_all(k_v.at[pl.ds(0, 8)], ksem.at[G])
          wait_all(v_v.at[pl.ds(0, 8)], vsem.at[G])
        @pl.when((h == 20) | (h == 22) | (h == 24) | (h == 25))
        def _():
          si = jnp.where(h <= 24, 3 + (h - 20) // 2, 6)
          wait_all(k_v.at[pl.ds(0, 2)], ksem.at[si])
          wait_all(v_v.at[pl.ds(0, 2)], vsem.at[si])
      with sc('b_head0'):
        if compute:
          nh = jnp.where(h < 20, 1, jnp.where(h < 26, 2, 0))
          def one(i, cc):
            idx = jnp.where(h < 24, h + 4 * i, 28 + 2 * (h - 24) + i)
            head(idx)
            return cc
          lax.fori_loop(0, nh, one, 0)
      return c
    with sc('s10_Bloop'):
      lax.fori_loop(0, NST, bh, 0)
    with sc('s11_bwo'):
      acc = jnp.zeros((8, 640), F32)
      for cch in range(4):
        wait_all(bwo_v.at[pl.ds(0, 1024)], sems.at[S_BWO0 + cch])
        if compute:
          for s in range(8):
            hd = s * 4 + cch
            acc = acc + jnp.dot(ob_s[hd].astype(BF), bwo_v[hd * 128:(hd + 1) * 128, :], preferred_element_type=F32)
      a_s2[...] = acc
    accB = a_s2[...]
    b_out = accB[0:1, :]
    a_out = jnp.sum(a_s[...], axis=0, keepdims=True)
    res = g * a_out + (1.0 - g) * b_out
    out_ref[0] = res.astype(out_ref.dtype)
  kernel.nsem = S_BWO0 + NCH
  return kernel


def build(compute=True, prof=False, cfg=None):
  kern = make_kernel(compute, prof, cfg)
  @jax.jit
  def fn(A_x, A_c_kv, A_w_q, A_w_uk, A_w_uv, A_w_o, B_x, B_k_cache, B_v_cache, B_wq, B_wo, gate_w):
    any_spec = pl.BlockSpec(memory_space=pl.ANY)
    V = pltpu.VMEM
    return pl.pallas_call(
        kern,
        in_specs=[any_spec] * 11,
        out_specs=pl.BlockSpec(memory_space=pltpu.VMEM),
        out_shape=jax.ShapeDtypeStruct((1, 1, 640), BF),
        scratch_shapes=[
            V((1, 1, 640), BF), V((640,), BF),
            V((4096, 512), BF), V((640 * 32, 128), BF), V((512 * 32, 128), BF), V((512 * 32, 128), BF),
            V((4096, 640), BF), V((32, 4096, 128), BF), V((32, 4096, 128), BF),
            V((640, 4096), BF), V((4096, 640), BF),
            V((160, 128), F32), V((32, 4096), F32),
            V((4, 8, 128), F32), V((32, 8, 128), F32), V((32, 8, 128), F32),
            V((32, 128), F32), V((128, 128), F32), V((32, 128), F32),
            V((128, 128), BF), V((8, 640), F32), V((8, 640), F32),
            pltpu.SemaphoreType.DMA((kern.nsem,)), pltpu.SemaphoreType.DMA((8,)), pltpu.SemaphoreType.DMA((8,)),
        ],
        compiler_params=pltpu.CompilerParams(vmem_limit_bytes=120 * 1024 * 1024),
    )(A_x, gate_w, A_c_kv.reshape(8, 512, 512), A_w_q.reshape(8, 2560, 128), A_w_uk.reshape(8, 2048, 128),
      A_w_uv.reshape(8, 2048, 128), A_w_o.reshape(8, 512, 640), B_k_cache.reshape(32, 4096, 128),
      B_v_cache.reshape(32, 4096, 128), B_wq.reshape(8, 80, 4096), B_wo.reshape(8, 512, 640))
  return fn

pallas_gated_mix__compressed_kv_cla__gqa_block_cached__decode_kernel = build(True)
```

```python
import jax
import jax.numpy as jnp
from jax import lax
from jax.experimental import pallas as pl
from jax.experimental.pallas import tpu as pltpu

BF = jnp.bfloat16
F32 = jnp.float32
I32 = jnp.int32
NT = (((1,), (1,)), ((), ()))

H, D, SK, M, DC = 32, 128, 4096, 640, 512
SCALE = D ** -0.5

S_X, S_G, S_WQ, S_BWQ, S_WUK, S_CKV, S_WUV, S_WO, S_BWO = range(9)
N_BWO_SEMS = 7
N_SEMS = S_BWO + N_BWO_SEMS


def _round_robin(n_streams, per_stream, make):
    return [make(s, k) for k in range(per_stream) for s in range(n_streams)]


def _interleave(a, b):
    assert len(a) == len(b)
    return [t for pair in zip(a, b) for t in pair]


def _iota(shape, dim):
    return lax.broadcasted_iota(I32, shape, dim)


def _kernel(x_hbm, gate_hbm, ckv_hbm, wq_hbm, wuk_hbm, wuv_hbm, wo_hbm, k_hbm, v_hbm, bwq_hbm, bwo_hbm,
            out_ref,
            x_v, gate_v, ckv_v, wq_v, wuk_v, wuv_v, wo_v, k_v, v_v, bwq_v, bwo_v,
            xe_s, qa_s, qabs_s, s_s, m_s, ct_s, ctx_s, a_s, qb_s, ob_s,
            sems, ksem, vsem):

    def start(src, dst, sem, thread):
        pltpu.make_async_copy(src, dst, sem).start(priority=thread)

    def wait_filled(dst, sem):
        pltpu.make_async_copy(dst, dst, sem).wait()

    def rows128(hbm, vmem, sem):
        per = vmem.shape[0] // 4

        def make(s, k):
            rows = pl.ds(s * per + k * 128, 128)
            return hbm.at[rows], vmem.at[rows], sems.at[sem]
        return _round_robin(4, per // 128, make)

    def bwq_descs():
        def make(s, k):
            rows, cols = pl.ds(s * 160 + (k // 2) * 8, 8), pl.ds((k % 2) * 2048, 2048)
            return bwq_hbm.at[rows, cols], bwq_v.at[rows, cols], sems.at[S_BWQ]
        return _round_robin(4, 40, make)

    def wide_rows(hbm, vmem, sem):
        def make(s, k):
            rows = pl.ds(s * 1024 + k * 32, 32)
            return hbm.at[rows], vmem.at[rows], sems.at[sem]
        return _round_robin(4, 32, make)

    def kv8_descs(group, first, count):
        heads = pl.ds(pl.multiple_of(8 * group, 8), 8) if not isinstance(group, int) else pl.ds(8 * group, 8)
        out = []
        for i in range(count):
            r0 = (first + i) * 16
            rows = pl.ds(r0, 16) if isinstance(r0, int) else pl.ds(pl.multiple_of(r0, 16), 16)
            out.append((k_hbm.at[heads, rows], k_v.at[heads, rows], ksem.at[group]))
            out.append((v_hbm.at[heads, rows], v_v.at[heads, rows], vsem.at[group]))
        return out

    k4_hbm, v4_hbm = k_hbm.reshape(2 * H, SK // 2, D), v_hbm.reshape(2 * H, SK // 2, D)
    k4_v, v4_v = k_v.reshape(2 * H, SK // 2, D), v_v.reshape(2 * H, SK // 2, D)

    def kv2_descs(pair, first, count, sem):
        segs = pl.ds(pl.multiple_of(4 * pair, 4), 4)
        out = []
        for i in range(count):
            rows = pl.ds(pl.multiple_of((first + i) * 32, 32), 32)
            out.append((k4_hbm.at[segs, rows], k4_v.at[segs, rows], ksem.at[sem]))
            out.append((v4_hbm.at[segs, rows], v4_v.at[segs, rows], vsem.at[sem]))
        return out

    def bwo_desc(s, k, sem):
        rows = pl.ds(s * 512 + k * 32, 32)
        return bwo_hbm.at[rows], bwo_v.at[rows], sems.at[sem]
    bwo_descs = [bwo_desc(s, k, S_BWO + k // 4) for k in range(12) for s in range(8)]
    bwo_descs += [bwo_desc(s, k, S_BWO + 3 + p) for p in range(4) for k in range(12, 16) for s in (2 * p, 2 * p + 1)]
    bwo3 = bwo_v.reshape(8, 512, M)

    phase0 = _interleave(rows128(wq_hbm, wq_v, S_WQ), bwq_descs())
    phase1 = _interleave(rows128(wuk_hbm, wuk_v, S_WUK), wide_rows(ckv_hbm, ckv_v, S_CKV))
    phase2 = _interleave(rows128(wuv_hbm, wuv_v, S_WUV), wide_rows(wo_hbm, wo_v, S_WO))
    stream = phase0 + phase1 + phase2 + kv8_descs(0, 0, 256)
    e0 = len(phase0)
    e1 = e0 + len(phase1)
    e2 = e1 + len(phase2)
    issued = [0]

    def issue(descs):
        for n, (src, dst, sem) in enumerate(descs):
            start(src, dst, sem, n % 2)

    def issue_to(target):
        assert issued[0] % 2 == 0
        issue(stream[issued[0]:target])
        issued[0] = max(issued[0], target)

    copy_x = pltpu.make_async_copy(x_hbm, x_v, sems.at[S_X])
    copy_g = pltpu.make_async_copy(gate_hbm, gate_v, sems.at[S_G])
    copy_x.start()
    copy_g.start()
    issue_to(88)
    copy_x.wait()
    copy_g.wait()

    xf = x_v[0].astype(F32)
    x8 = jnp.broadcast_to(xf, (8, M)).astype(BF)
    gate_prod = (xf * gate_v[...].astype(F32).reshape(1, M)).astype(BF).astype(F32)
    gate = jax.nn.sigmoid(jnp.sum(gate_prod, axis=-1, keepdims=True))

    sel_t = jnp.where(_iota((160, M), 1) // 4 == _iota((160, M), 0),
                      jnp.broadcast_to(xf, (160, M)), 0.0).astype(BF)
    sel_l = (_iota((M, 128), 0) % 4 == _iota((M, 128), 1) // 32).astype(F32).astype(BF)
    xe_s[...] = jnp.dot(sel_t, sel_l, preferred_element_type=F32)
    qa_s[...] = jnp.zeros(qa_s.shape, F32)
    qabs_s[...] = jnp.zeros(qabs_s.shape, F32)

    def head_diag():
        return _iota((H, 128), 0) == _iota((H, 128), 1) % H

    def qa_part(i0, i1):
        diag = head_diag()
        acc = qa_s[...]
        for it in range(i0, i1):
            xe8 = xe_s[it * 8:(it + 1) * 8, :]
            lhs = jnp.concatenate(
                [jnp.where(diag, jnp.broadcast_to(xe8[t:t + 1, :], (H, 128)), 0.0).astype(BF) for t in range(8)],
                axis=1)
            acc = acc + jnp.dot(lhs, wq_v[it * 1024:(it + 1) * 1024, :], preferred_element_type=F32)
        qa_s[...] = acc

    def qb_part():
        for c in range(4):
            qb = jnp.dot(x8, bwq_v[:, c * 1024:(c + 1) * 1024], preferred_element_type=F32)
            for hh in range(8):
                qb_s[c * 8 + hh] = qb[:, hh * D:(hh + 1) * D]

    def qabs_part(t0, t1):
        diag = head_diag()
        col = _iota((128, 128), 1) - _iota((128, 128), 0) // H
        q = qa_s[...].astype(BF)
        acc = qabs_s[...]
        for t in range(t0, t1):
            picked = []
            for ch in range(4):
                tile = wuk_v[ch * 4096 + t * 128:ch * 4096 + (t + 1) * 128, :]
                r = lax.dot_general(q, tile, NT, preferred_element_type=F32)
                picked.append(jnp.where(diag, r, 0.0).astype(BF))
            gather = (col == 4 * t).astype(F32).astype(BF)
            acc = acc + jnp.dot(jnp.concatenate(picked, axis=0), gather, preferred_element_type=F32)
        qabs_s[...] = acc

    kc = 512

    def scores_part():
        acc = qabs_s[...]
        qabs = jnp.concatenate([acc[ch * H:(ch + 1) * H, :] for ch in range(4)], axis=1).astype(BF)
        m = jnp.full((H, 1), -jnp.inf, F32)
        for i in range(SK // kc):
            s = lax.dot_general(qabs, ckv_v[i * kc:(i + 1) * kc, :], NT, preferred_element_type=F32) * SCALE
            s_s[:, i * kc:(i + 1) * kc] = s
            m = jnp.maximum(m, jnp.max(s, axis=1, keepdims=True))
        m_s[...] = jnp.broadcast_to(m, (H, 128))

    def ctxc_part():
        m = m_s[:, 0:1]
        l = jnp.zeros((H, 1), F32)
        acc = jnp.zeros((H, DC), F32)
        for i in range(SK // kc):
            p = jnp.exp(s_s[:, i * kc:(i + 1) * kc] - m)
            l = l + jnp.sum(p, axis=1, keepdims=True)
            acc = acc + jnp.dot(p.astype(BF), ckv_v[i * kc:(i + 1) * kc, :], preferred_element_type=F32)
        ctxc = (acc / l).astype(BF)
        ct_s[...] = jnp.concatenate([ctxc[:, ch * 128:(ch + 1) * 128] for ch in range(4)], axis=0)

    def ctx_part(t0, t1):
        diag = head_diag()
        row = _iota((128, 128), 0) - _iota((128, 128), 1) // H
        ct = ct_s[...]
        acc = jnp.zeros((H, D), F32)
        for t in range(t0, t1):
            spread = (row == 4 * t).astype(F32).astype(BF)
            z = jnp.dot(ct, spread, preferred_element_type=F32)
            for ch in range(4):
                lhs = jnp.where(diag, z[ch * H:(ch + 1) * H, :], 0.0).astype(BF)
                tile = wuv_v[ch * 4096 + t * 128:ch * 4096 + (t + 1) * 128, :]
                acc = acc + jnp.dot(lhs, tile, preferred_element_type=F32)
        if t0 == 0:
            ctx_s[...] = acc.reshape(4, 8, D)
        else:
            ctx_s[...] = ctx_s[...] + acc.reshape(4, 8, D)

    def outa_part():
        row8 = _iota((8, D), 0)
        acc = jnp.zeros((8, M), F32)
        for gi in range(4):
            cg = ctx_s[gi]
            lhs = jnp.concatenate([jnp.where(row8 == hh, cg, 0.0).astype(BF) for hh in range(8)], axis=1)
            acc = acc + jnp.dot(lhs, wo_v[gi * 1024:(gi + 1) * 1024, :], preferred_element_type=F32)
        a_s[...] = acc

    def wait_phase0():
        wait_filled(wq_v, sems.at[S_WQ])
        wait_filled(bwq_v, sems.at[S_BWQ])

    def wait_phase1():
        wait_filled(wuk_v, sems.at[S_WUK])
        wait_filled(ckv_v, sems.at[S_CKV])

    def wait_phase2():
        wait_filled(wuv_v, sems.at[S_WUV])
        wait_filled(wo_v, sems.at[S_WO])

    slots = [
        (e0, None, None),
        (e0 + 112, wait_phase0, lambda: qa_part(0, 10)),
        (e0 + 152, None, lambda: qa_part(10, 20)),
        (e0 + 192, None, qb_part),
        (e1, None, None),
        (e1 + 112, wait_phase1, lambda: qabs_part(0, 16)),
        (e1 + 152, None, lambda: qabs_part(16, 32)),
        (e1 + 192, None, scores_part),
        (e1 + 232, None, ctxc_part),
        (e2, None, None),
        (e2 + 112, wait_phase2, lambda: ctx_part(0, 16)),
        (e2 + 144, None, lambda: ctx_part(16, 32)),
        (e2 + 176, None, outa_part),
        (len(stream), None, None),
    ]

    def run_slot(k, carry):
        for n, (target, wait, stage) in enumerate(slots):
            @pl.when(k == n)
            def _(target=target, wait=wait, stage=stage):
                issue_to(target)
                if wait is not None:
                    wait()
                if stage is not None:
                    stage()
        return carry

    lax.fori_loop(0, len(slots), run_slot, 0)
    assert issued[0] == len(stream)

    def head(h):
        q = qb_s[h].astype(BF)
        s = lax.dot_general(q, k_v[h], NT, preferred_element_type=F32) * SCALE
        m = jnp.max(s, axis=1, keepdims=True)
        p = jnp.exp(s - m)
        l = jnp.sum(p, axis=1, keepdims=True)
        ob_s[h] = jnp.dot(p.astype(BF), v_v[h], preferred_element_type=F32) / l

    def step(h, carry):
        group = h // 8
        hh = h % 8

        @pl.when(h < 16)
        def _():
            issue(kv8_descs(group + 1, hh * 32, 32))

        @pl.when((h >= 16) & (h < 24))
        def _():
            j = h - 16
            issue(kv2_descs(12 + j // 2, (j % 2) * 32, 32, 3 + j // 2))

        for n in range(2):
            @pl.when(h == 24 + n)
            def _(n=n):
                issue(bwo_descs[64 * n:64 * (n + 1)])

        @pl.when((hh == 0) & (h < 24))
        def _():
            heads = pl.ds(pl.multiple_of(8 * group, 8), 8)
            wait_filled(k_v.at[heads], ksem.at[group])
            wait_filled(v_v.at[heads], vsem.at[group])

        @pl.when((h == 20) | (h == 22) | (h == 24) | (h == 25))
        def _():
            pair = jnp.where(h <= 24, (h - 20) // 2, 3)
            heads = pl.ds(pl.multiple_of(24 + 2 * pair, 2), 2)
            wait_filled(k_v.at[heads], ksem.at[3 + pair])
            wait_filled(v_v.at[heads], vsem.at[3 + pair])

        n_heads = jnp.where(h < 20, 1, 2)

        def one(i, c):
            head(jnp.where(h < 24, h + 4 * i, 28 + 2 * (h - 24) + i))
            return c
        lax.fori_loop(0, n_heads, one, 0)
        return carry

    lax.fori_loop(0, 26, step, 0)

    def out_proj(acc, hd):
        w = bwo_v[hd * D:(hd + 1) * D, :]
        return acc + jnp.dot(ob_s[hd].astype(BF), w, preferred_element_type=F32)

    acc_b = jnp.zeros((8, M), F32)
    for c in range(3):
        wait_filled(bwo3.at[:, pl.ds(c * D, D)], sems.at[S_BWO + c])
        for s in range(8):
            acc_b = out_proj(acc_b, 4 * s + c)
    for p in range(4):
        wait_filled(bwo3.at[pl.ds(2 * p, 2), pl.ds(3 * D, D)], sems.at[S_BWO + 3 + p])
        for s in (2 * p, 2 * p + 1):
            acc_b = out_proj(acc_b, 4 * s + 3)

    a_out = jnp.sum(a_s[...], axis=0, keepdims=True)
    res = gate * a_out + (1.0 - gate) * acc_b[0:1, :]
    out_ref[0] = res.astype(out_ref.dtype)


@jax.jit
def pallas_gated_mix__compressed_kv_cla__gqa_block_cached__decode_kernel(
    A_x: jax.Array,
    A_c_kv: jax.Array,
    A_w_q: jax.Array,
    A_w_uk: jax.Array,
    A_w_uv: jax.Array,
    A_w_o: jax.Array,
    B_x: jax.Array,
    B_k_cache: jax.Array,
    B_v_cache: jax.Array,
    B_wq: jax.Array,
    B_wo: jax.Array,
    gate_w: jax.Array,
):
    del B_x
    hbm = pl.BlockSpec(memory_space=pl.ANY)
    vmem = pltpu.VMEM
    return pl.pallas_call(
        _kernel,
        in_specs=[hbm] * 11,
        out_specs=pl.BlockSpec(memory_space=pltpu.VMEM),
        out_shape=jax.ShapeDtypeStruct((1, 1, M), BF),
        scratch_shapes=[
            vmem((1, 1, M), BF),
            vmem((M,), BF),
            vmem((SK, DC), BF),
            vmem((M * H, D), BF),
            vmem((DC * H, D), BF),
            vmem((DC * H, D), BF),
            vmem((H * D, M), BF),
            vmem((H, SK, D), BF),
            vmem((H, SK, D), BF),
            vmem((M, H * D), BF),
            vmem((H * D, M), BF),
            vmem((160, 128), F32),
            vmem((H, D), F32),
            vmem((128, 128), F32),
            vmem((H, SK), F32),
            vmem((H, 128), F32),
            vmem((128, 128), BF),
            vmem((4, 8, D), F32),
            vmem((8, M), F32),
            vmem((H, 8, D), F32),
            vmem((H, 8, D), F32),
            pltpu.SemaphoreType.DMA((N_SEMS,)),
            pltpu.SemaphoreType.DMA((7,)),
            pltpu.SemaphoreType.DMA((7,)),
        ],
        compiler_params=pltpu.CompilerParams(vmem_limit_bytes=120 * 1024 * 1024),
    )(A_x, gate_w, A_c_kv.reshape(SK, DC), A_w_q.reshape(M * H, D), A_w_uk.reshape(DC * H, D),
      A_w_uv.reshape(DC * H, D), A_w_o.reshape(H * D, M), B_k_cache.reshape(H, SK, D),
      B_v_cache.reshape(H, SK, D), B_wq, B_wo)
```

```python
import jax
import jax.numpy as jnp
from jax import lax
from jax.experimental import pallas as pl
from jax.experimental.pallas import tpu as pltpu

BF = jnp.bfloat16
F32 = jnp.float32
I32 = jnp.int32
NT = (((1,), (1,)), ((), ()))

H, D, SK, M, DC = 32, 128, 4096, 640, 512
SCALE = D ** -0.5

S_X, S_G, S_WQ, S_BWQ, S_WUK, S_CKV, S_WUV, S_WO, S_BWO = range(9)
N_BWO_SEMS = 7
N_SEMS = S_BWO + N_BWO_SEMS


def _round_robin(n_streams, per_stream, make):
    return [make(s, k) for k in range(per_stream) for s in range(n_streams)]


def _interleave(a, b):
    assert len(a) == len(b)
    return [t for pair in zip(a, b) for t in pair]


def _iota(shape, dim):
    return lax.broadcasted_iota(I32, shape, dim)


def _kernel(x_hbm, gate_hbm, ckv_hbm, wq_hbm, wuk_hbm, wuv_hbm, wo_hbm, k_hbm, v_hbm, bwq_hbm, bwo_hbm,
            out_ref,
            x_v, gate_v, ckv_v, wq_v, wuk_v, wuv_v, wo_v, k_v, v_v, bwq_v, bwo_v,
            xe_s, qa_s, qabs_s, s_s, m_s, ct_s, ctx_s, a_s, qb_s, ob_s,
            sems, ksem, vsem):

    def start(src, dst, sem, thread):
        pltpu.make_async_copy(src, dst, sem).start(priority=thread)

    def wait_filled(dst, sem):
        pltpu.make_async_copy(dst, dst, sem).wait()

    def rows128(hbm, vmem, sem):
        per = vmem.shape[0] // 4

        def make(s, k):
            rows = pl.ds(s * per + k * 128, 128)
            return hbm.at[rows], vmem.at[rows], sems.at[sem]
        return _round_robin(4, per // 128, make)

    def bwq_descs():
        def make(s, k):
            rows, cols = pl.ds(s * 160 + (k // 2) * 8, 8), pl.ds((k % 2) * 2048, 2048)
            return bwq_hbm.at[rows, cols], bwq_v.at[rows, cols], sems.at[S_BWQ]
        return _round_robin(4, 40, make)

    def wide_rows(hbm, vmem, sem):
        def make(s, k):
            rows = pl.ds(s * 1024 + k * 32, 32)
            return hbm.at[rows], vmem.at[rows], sems.at[sem]
        return _round_robin(4, 32, make)

    def kv8_descs(group, first, count):
        heads = pl.ds(pl.multiple_of(8 * group, 8), 8) if not isinstance(group, int) else pl.ds(8 * group, 8)
        out = []
        for i in range(count):
            r0 = (first + i) * 16
            rows = pl.ds(r0, 16) if isinstance(r0, int) else pl.ds(pl.multiple_of(r0, 16), 16)
            out.append((k_hbm.at[heads, rows], k_v.at[heads, rows], ksem.at[group]))
            out.append((v_hbm.at[heads, rows], v_v.at[heads, rows], vsem.at[group]))
        return out

    def kv4_descs(quad, first, count, sem):
        heads = pl.ds(pl.multiple_of(4 * quad, 4), 4)
        out = []
        for i in range(count):
            rows = pl.ds(pl.multiple_of((first + i) * 32, 32), 32)
            out.append((k_hbm.at[heads, rows], k_v.at[heads, rows], ksem.at[sem]))
            out.append((v_hbm.at[heads, rows], v_v.at[heads, rows], vsem.at[sem]))
        return out

    def bwo_desc(s, k, sem):
        rows = pl.ds(k * 32, 32)
        return bwo_hbm.at[s, rows], bwo_v.at[s, rows], sems.at[sem]
    bwo_descs = [bwo_desc(s, k, S_BWO + k // 4) for k in range(12) for s in range(8)]
    bwo_descs += [bwo_desc(s, k, S_BWO + 3 + p) for p in range(4) for k in range(12, 16) for s in (2 * p, 2 * p + 1)]

    phase0 = _interleave(rows128(wq_hbm, wq_v, S_WQ), bwq_descs())
    phase1 = _interleave(rows128(wuk_hbm, wuk_v, S_WUK), wide_rows(ckv_hbm, ckv_v, S_CKV))
    phase2 = _interleave(rows128(wuv_hbm, wuv_v, S_WUV), wide_rows(wo_hbm, wo_v, S_WO))
    stream = phase0 + phase1 + phase2 + kv8_descs(0, 0, 256)
    e0 = len(phase0)
    e1 = e0 + len(phase1)
    e2 = e1 + len(phase2)
    issued = [0]

    def issue(descs):
        for n, (src, dst, sem) in enumerate(descs):
            start(src, dst, sem, n % 2)

    def issue_to(target):
        assert issued[0] % 2 == 0
        issue(stream[issued[0]:target])
        issued[0] = max(issued[0], target)

    copy_x = pltpu.make_async_copy(x_hbm, x_v, sems.at[S_X])
    copy_g = pltpu.make_async_copy(gate_hbm, gate_v, sems.at[S_G])
    copy_x.start()
    copy_g.start()
    issue_to(88)
    copy_x.wait()
    copy_g.wait()

    xf = x_v[0].astype(F32)
    x8 = jnp.broadcast_to(xf, (8, M)).astype(BF)
    gate_prod = (xf * gate_v[...].astype(F32).reshape(1, M)).astype(BF).astype(F32)
    gate = jax.nn.sigmoid(jnp.sum(gate_prod, axis=-1, keepdims=True))

    sel_t = jnp.where(_iota((160, M), 1) // 4 == _iota((160, M), 0),
                      jnp.broadcast_to(xf, (160, M)), 0.0).astype(BF)
    sel_l = (_iota((M, 128), 0) % 4 == _iota((M, 128), 1) // 32).astype(F32).astype(BF)
    xe_s[...] = jnp.dot(sel_t, sel_l, preferred_element_type=F32)
    qa_s[...] = jnp.zeros(qa_s.shape, F32)
    qabs_s[...] = jnp.zeros(qabs_s.shape, F32)

    def head_diag():
        return _iota((H, 128), 0) == _iota((H, 128), 1) % H

    def qa_part(i0, i1):
        diag = head_diag()
        acc = qa_s[...]
        for it in range(i0, i1):
            xe8 = xe_s[it * 8:(it + 1) * 8, :]
            lhs = jnp.concatenate(
                [jnp.where(diag, jnp.broadcast_to(xe8[t:t + 1, :], (H, 128)), 0.0).astype(BF) for t in range(8)],
                axis=1)
            acc = acc + jnp.dot(lhs, wq_v[it * 1024:(it + 1) * 1024, :], preferred_element_type=F32)
        qa_s[...] = acc

    def qb_part():
        for c in range(4):
            qb = jnp.dot(x8, bwq_v[:, c * 1024:(c + 1) * 1024], preferred_element_type=F32)
            for hh in range(8):
                qb_s[c * 8 + hh] = qb[:, hh * D:(hh + 1) * D]

    def qabs_part(t0, t1):
        diag = head_diag()
        col = _iota((128, 128), 1) - _iota((128, 128), 0) // H
        q = qa_s[...].astype(BF)
        acc = qabs_s[...]
        for t in range(t0, t1):
            picked = []
            for ch in range(4):
                tile = wuk_v[ch * 4096 + t * 128:ch * 4096 + (t + 1) * 128, :]
                r = lax.dot_general(q, tile, NT, preferred_element_type=F32)
                picked.append(jnp.where(diag, r, 0.0).astype(BF))
            gather = (col == 4 * t).astype(F32).astype(BF)
            acc = acc + jnp.dot(jnp.concatenate(picked, axis=0), gather, preferred_element_type=F32)
        qabs_s[...] = acc

    kc = 512

    def scores_part():
        acc = qabs_s[...]
        qabs = jnp.concatenate([acc[ch * H:(ch + 1) * H, :] for ch in range(4)], axis=1).astype(BF)
        m = jnp.full((H, 1), -jnp.inf, F32)
        for i in range(SK // kc):
            s = lax.dot_general(qabs, ckv_v[i * kc:(i + 1) * kc, :], NT, preferred_element_type=F32) * SCALE
            s_s[:, i * kc:(i + 1) * kc] = s
            m = jnp.maximum(m, jnp.max(s, axis=1, keepdims=True))
        m_s[...] = jnp.broadcast_to(m, (H, 128))

    def ctxc_part():
        m = m_s[:, 0:1]
        l = jnp.zeros((H, 1), F32)
        acc = jnp.zeros((H, DC), F32)
        for i in range(SK // kc):
            p = jnp.exp(s_s[:, i * kc:(i + 1) * kc] - m)
            l = l + jnp.sum(p, axis=1, keepdims=True)
            acc = acc + jnp.dot(p.astype(BF), ckv_v[i * kc:(i + 1) * kc, :], preferred_element_type=F32)
        ctxc = (acc / l).astype(BF)
        ct_s[...] = jnp.concatenate([ctxc[:, ch * 128:(ch + 1) * 128] for ch in range(4)], axis=0)

    def ctx_part(t0, t1):
        diag = head_diag()
        row = _iota((128, 128), 0) - _iota((128, 128), 1) // H
        ct = ct_s[...]
        acc = jnp.zeros((H, D), F32)
        for t in range(t0, t1):
            spread = (row == 4 * t).astype(F32).astype(BF)
            z = jnp.dot(ct, spread, preferred_element_type=F32)
            for ch in range(4):
                lhs = jnp.where(diag, z[ch * H:(ch + 1) * H, :], 0.0).astype(BF)
                tile = wuv_v[ch * 4096 + t * 128:ch * 4096 + (t + 1) * 128, :]
                acc = acc + jnp.dot(lhs, tile, preferred_element_type=F32)
        if t0 == 0:
            ctx_s[...] = acc.reshape(4, 8, D)
        else:
            ctx_s[...] = ctx_s[...] + acc.reshape(4, 8, D)

    def outa_part():
        row8 = _iota((8, D), 0)
        acc = jnp.zeros((8, M), F32)
        for gi in range(4):
            cg = ctx_s[gi]
            lhs = jnp.concatenate([jnp.where(row8 == hh, cg, 0.0).astype(BF) for hh in range(8)], axis=1)
            acc = acc + jnp.dot(lhs, wo_v[gi * 1024:(gi + 1) * 1024, :], preferred_element_type=F32)
        a_s[...] = acc

    def wait_phase0():
        wait_filled(wq_v, sems.at[S_WQ])
        wait_filled(bwq_v, sems.at[S_BWQ])

    def wait_phase1():
        wait_filled(wuk_v, sems.at[S_WUK])
        wait_filled(ckv_v, sems.at[S_CKV])

    def wait_phase2():
        wait_filled(wuv_v, sems.at[S_WUV])
        wait_filled(wo_v, sems.at[S_WO])

    slots = [
        (e0, None, None),
        (e0 + 112, wait_phase0, lambda: qa_part(0, 10)),
        (e0 + 152, None, lambda: qa_part(10, 20)),
        (e0 + 192, None, qb_part),
        (e1, None, None),
        (e1 + 112, wait_phase1, lambda: qabs_part(0, 16)),
        (e1 + 152, None, lambda: qabs_part(16, 32)),
        (e1 + 192, None, scores_part),
        (e1 + 232, None, ctxc_part),
        (e2, None, None),
        (e2 + 112, wait_phase2, lambda: ctx_part(0, 16)),
        (e2 + 144, None, lambda: ctx_part(16, 32)),
        (e2 + 176, None, outa_part),
        (len(stream), None, None),
    ]

    def run_slot(k, carry):
        for n, (target, wait, stage) in enumerate(slots):
            @pl.when(k == n)
            def _(target=target, wait=wait, stage=stage):
                issue_to(target)
                if wait is not None:
                    wait()
                if stage is not None:
                    stage()
        return carry

    lax.fori_loop(0, len(slots), run_slot, 0)
    assert issued[0] == len(stream)

    def head(h):
        q = qb_s[h].astype(BF)
        s = lax.dot_general(q, k_v[h], NT, preferred_element_type=F32) * SCALE
        m = jnp.max(s, axis=1, keepdims=True)
        p = jnp.exp(s - m)
        l = jnp.sum(p, axis=1, keepdims=True)
        ob_s[h] = jnp.dot(p.astype(BF), v_v[h], preferred_element_type=F32) / l

    def step(h, carry):
        group = h // 8
        hh = h % 8

        @pl.when(h < 16)
        def _():
            issue(kv8_descs(group + 1, hh * 32, 32))

        @pl.when((h >= 16) & (h < 24))
        def _():
            j = h - 16
            issue(kv4_descs(6 + j // 4, (j % 4) * 32, 32, 3 + j // 4))

        for n in range(2):
            @pl.when(h == 24 + n)
            def _(n=n):
                issue(bwo_descs[64 * n:64 * (n + 1)])

        @pl.when((hh == 0) & (h < 24))
        def _():
            heads = pl.ds(pl.multiple_of(8 * group, 8), 8)
            wait_filled(k_v.at[heads], ksem.at[group])
            wait_filled(v_v.at[heads], vsem.at[group])

        @pl.when((h == 21) | (h == 25))
        def _():
            quad = (h - 21) // 4
            heads = pl.ds(pl.multiple_of(24 + 4 * quad, 4), 4)
            wait_filled(k_v.at[heads], ksem.at[3 + quad])
            wait_filled(v_v.at[heads], vsem.at[3 + quad])

        n_heads = jnp.where(h <= 20, 1, jnp.where(h <= 23, 2, jnp.where(h == 24, 1, 4)))

        def one(i, c):
            head(jnp.where(h <= 23, h + 3 * i, jnp.where(h == 24, 27, 28 + i)))
            return c
        lax.fori_loop(0, n_heads, one, 0)
        return carry

    lax.fori_loop(0, 26, step, 0)

    def out_proj(acc, s, c):
        w = bwo_v[s, c * D:(c + 1) * D, :]
        return acc + jnp.dot(ob_s[4 * s + c].astype(BF), w, preferred_element_type=F32)

    acc_b = jnp.zeros((8, M), F32)
    for c in range(3):
        wait_filled(bwo_v.at[:, pl.ds(c * D, D)], sems.at[S_BWO + c])
        for s in range(8):
            acc_b = out_proj(acc_b, s, c)
    for p in range(4):
        wait_filled(bwo_v.at[pl.ds(2 * p, 2), pl.ds(3 * D, D)], sems.at[S_BWO + 3 + p])
        for s in (2 * p, 2 * p + 1):
            acc_b = out_proj(acc_b, s, 3)

    a_out = jnp.sum(a_s[...], axis=0, keepdims=True)
    res = gate * a_out + (1.0 - gate) * acc_b[0:1, :]
    out_ref[0] = res.astype(out_ref.dtype)


@jax.jit
def pallas_gated_mix__compressed_kv_cla__gqa_block_cached__decode_kernel(
    A_x: jax.Array,
    A_c_kv: jax.Array,
    A_w_q: jax.Array,
    A_w_uk: jax.Array,
    A_w_uv: jax.Array,
    A_w_o: jax.Array,
    B_x: jax.Array,
    B_k_cache: jax.Array,
    B_v_cache: jax.Array,
    B_wq: jax.Array,
    B_wo: jax.Array,
    gate_w: jax.Array,
):
    del B_x
    hbm = pl.BlockSpec(memory_space=pl.ANY)
    vmem = pltpu.VMEM
    return pl.pallas_call(
        _kernel,
        in_specs=[hbm] * 11,
        out_specs=pl.BlockSpec(memory_space=pltpu.VMEM),
        out_shape=jax.ShapeDtypeStruct((1, 1, M), BF),
        scratch_shapes=[
            vmem((1, 1, M), BF),
            vmem((M,), BF),
            vmem((SK, DC), BF),
            vmem((M * H, D), BF),
            vmem((DC * H, D), BF),
            vmem((DC * H, D), BF),
            vmem((H * D, M), BF),
            vmem((H, SK, D), BF),
            vmem((H, SK, D), BF),
            vmem((M, H * D), BF),
            vmem((8, 4 * D, M), BF),
            vmem((160, 128), F32),
            vmem((H, D), F32),
            vmem((128, 128), F32),
            vmem((H, SK), F32),
            vmem((H, 128), F32),
            vmem((128, 128), BF),
            vmem((4, 8, D), F32),
            vmem((8, M), F32),
            vmem((H, 8, D), F32),
            vmem((H, 8, D), F32),
            pltpu.SemaphoreType.DMA((N_SEMS,)),
            pltpu.SemaphoreType.DMA((5,)),
            pltpu.SemaphoreType.DMA((5,)),
        ],
        compiler_params=pltpu.CompilerParams(vmem_limit_bytes=120 * 1024 * 1024),
    )(A_x, gate_w, A_c_kv.reshape(SK, DC), A_w_q.reshape(M * H, D), A_w_uk.reshape(DC * H, D),
      A_w_uv.reshape(DC * H, D), A_w_o.reshape(H * D, M), B_k_cache.reshape(H, SK, D),
      B_v_cache.reshape(H, SK, D), B_wq, B_wo.reshape(8, 4 * D, M))
```
